```python
import jax
import jax.numpy as jnp

def _softmax(x, axis=-1):
    return jax.nn.softmax(x, axis=axis)
def _gelu(x):
    return jax.nn.gelu(x, approximate=True)
def _silu(x):
    return jax.nn.silu(x)
def _sigmoid(x):
    return jax.nn.sigmoid(x)
def _layernorm(x, axis=-1, eps=1e-5):
    m = jnp.mean(x, axis=axis, keepdims=True)
    v = jnp.var(x, axis=axis, keepdims=True)
    return (x - m) / jnp.sqrt(v + eps)
def _scatter_add(tgt, idx, src, axis=0):
    return tgt.at[idx].add(src)
def _segment_sum(src, seg, n):
    return jax.ops.segment_sum(src, seg, n)
class _Rng:
    def __init__(self, key):
        self._k = key
    def _next(self):
        self._k, sub = jax.random.split(self._k)
        return sub
    def normal(self, shape):
        return jax.random.normal(self._next(), shape, dtype=jnp.bfloat16)
    def randint(self, lo, hi, shape):
        return jax.random.randint(self._next(), shape, lo, hi, dtype=jnp.int32)
    def uniform(self, shape, lo=0.0, hi=1.0):
        return jax.random.uniform(self._next(), shape, jnp.bfloat16, lo, hi)
    def permutation(self, n):
        return jax.random.permutation(self._next(), n)


kernel_name = 'recurrent_scan__gqa_block_cached__moe_arch_mod__prompt'

def setup_inputs():
    _rng = _Rng(jax.random.key(int.from_bytes(__import__("os").urandom(4), "little")))
    _w = (lambda a: (lambda t: t.astype(jnp.bfloat16) if jnp.issubdtype(t.dtype, jnp.floating) else t)(jnp.asarray(a)))
    def _A_setup():
        B, Sq, D = 1, 2048, 576
        Hq, Hkv, Sk, Dh = 32, 16, 2048, 128
        assert Hq % Hkv == 0, (Hq, Hkv)
        return {
            "x": _w((lambda *s: _rng.normal(s) * 0.05)(B, Sq, D)),
            "k_cache": _w((lambda *s: _rng.normal(s) * 0.05)(B, Hkv, Sk, Dh)),
            "v_cache": _w((lambda *s: _rng.normal(s) * 0.05)(B, Hkv, Sk, Dh)),
            "wq": _w((lambda *s: _rng.normal(s) * 0.05)(D, Hq * Dh) * (D ** -0.5)),
            "wo": _w((lambda *s: _rng.normal(s) * 0.05)(Hq * Dh, D) * ((Hq * Dh) ** -0.5)),
        }
    _A_in = _A_setup()

    def _B_setup():
        B, S, D, F, C = 1, 2048, 576, 4608, 8
        return {
            "x": _w((lambda *s: _rng.normal(s) * 0.05)(B, S, D)),
            "w_r": _w((lambda *s: _rng.normal(s) * 0.05)(D)),
            "w_gate": _w((lambda *s: _rng.normal(s) * 0.05)(D, F)),
            "w_up": _w((lambda *s: _rng.normal(s) * 0.05)(D, F)),
            "w_down": _w((lambda *s: _rng.normal(s) * 0.05)(F, D)),
        }
    _B_in = _B_setup()

    return {
        "A_x": _A_in["x"],
        "A_k_cache": _A_in["k_cache"],
        "A_v_cache": _A_in["v_cache"],
        "A_wq": _A_in["wq"],
        "A_wo": _A_in["wo"],
        "B_x": _B_in["x"],
        "B_w_r": _B_in["w_r"],
        "B_w_gate": _B_in["w_gate"],
        "B_w_up": _B_in["w_up"],
        "B_w_down": _B_in["w_down"],
    }

def reference(A_x, A_k_cache, A_v_cache, A_wq, A_wo, B_x, B_w_r, B_w_gate, B_w_up, B_w_down):
    def _A_ref(x, k_cache, v_cache, wq, wo):
        B, Sq, D = x.shape
        Hq, Dh = 32, 128
        Hkv = k_cache.shape[1]
        rep = Hq // Hkv
        q = (lambda x, *d: x.transpose(*d))((x @ wq).reshape(B, Sq, Hq, Dh), 0, 2, 1, 3)
        k = jnp.repeat(k_cache, rep, axis=1)
        v = jnp.repeat(v_cache, rep, axis=1)
        scores = jnp.einsum("bhqd,bhkd->bhqk", q, k) * (Dh ** -0.5)
        p = _softmax(scores, axis=-1)
        o = jnp.einsum("bhqk,bhkd->bhqd", p, v)
        return (lambda x, *d: x.transpose(*d))(o, 0, 2, 1, 3).reshape(B, Sq, Hq * Dh) @ wo

    def _B_ref(x, w_r, w_gate, w_up, w_down):
        B, S, D = x.shape
        C = 8
        r = x @ w_r
        idx = jnp.argsort(-r, axis=-1)[:, :C]
        idx_e = jnp.repeat(idx.reshape(B, C, 1), D, axis=2)
        x_sel = jnp.take_along_axis(x, idx_e, axis=1)
        g = _silu(x_sel @ w_gate)
        u = x_sel @ w_up
        y = (g * u) @ w_down
        r_sel = _sigmoid(jnp.take_along_axis(r, idx, axis=1))
        y = y * r_sel.reshape(B, C, 1)
        b_off = (jnp.arange(B) * S).reshape(B, 1)
        flat_idx = (idx + b_off).reshape(B * C)
        zero = (x * 0.0).reshape(B * S, D)
        upd = _scatter_add(zero, flat_idx, y.reshape(B * C, D), axis=0)
        return x + upd.reshape(B, S, D)

    x = A_x
    xn = _layernorm(x, axis=-1)
    s = _A_ref(xn, A_k_cache, A_v_cache, A_wq, A_wo)
    g = _silu(_B_ref(xn, B_w_r, B_w_gate, B_w_up, B_w_down))
    return x + s * g
```

```python
import functools
import jax
import jax.numpy as jnp
from jax import lax
import jax.experimental.pallas as pl
import jax.experimental.pallas.tpu as pltpu

S = 2048
D = 576
DP = 640
HQ = 32
HKV = 16
DH = 128
F = 4608
C = 8
LOG2E = 1.4426950408889634
QSCALE = (DH ** -0.5) * LOG2E
bf16 = jnp.bfloat16
f32 = jnp.float32
u32 = jnp.uint32
NT = (((1,), (1,)), ((), ()))


def _rb(x):
    return x.astype(bf16).astype(f32)


def _pk(x):
    return pltpu.bitcast(x, u32)


def _upk(x):
    return pltpu.bitcast(x, bf16)


def _tree(p, op):
    parts = [p[i * 8:(i + 1) * 8] for i in range(p.shape[0] // 8)]
    while len(parts) > 1:
        parts = [op(parts[i], parts[i + 1]) for i in range(0, len(parts), 2)]
    return parts[0]


def make_kernel(MQ=512, KBQ=2048, KBP=512, VL=110, order="qa,qb,op,pa,qp,pb,vt", MOE_T=8, MOE_DMA_T=1,
                gate=True):
    NQ = S // MQ
    NL = S // 128
    NTQ = MQ // 128
    T = HKV * NQ
    VP = S // NQ
    NKT = S // 128

    def kernel(xt_hbm, k_hbm, v_hbm, wq_hbm, wot_hbm, wr_ref, wg_hbm, wu_hbm, wdt_hbm,
               o_hbm,
               xn_ref, acc_ref, k_ref, v_ref, wq_ref, wo_ref,
               sa_ref, sb_ref, q_ref, oc_ref, vt_ref,
               bt_ref, xs_ref, r_ref, wrb_ref, wg_ref, wu_ref, wdt_ref, z_ref,
               sem_x, sem_k, sem_v, sem_wq, sem_wo, sem_m, sem_o):

        def cp_x(ib):
            return pltpu.make_async_copy(xt_hbm.at[:, pl.ds(ib * MQ, MQ)], xs_ref.at[ib], sem_x.at[ib])

        def cp_k(h):
            return pltpu.make_async_copy(k_hbm.at[0, h], k_ref.at[h], sem_k.at[h])

        def cp_v(h):
            return pltpu.make_async_copy(v_hbm.at[0, h], v_ref.at[h], sem_v.at[h])

        def cp_wq(h):
            return pltpu.make_async_copy(wq_hbm.at[:, pl.ds(pl.multiple_of(h * 256, 256), 256)], wq_ref.at[h], sem_wq.at[h])

        def cp_wo(h):
            return pltpu.make_async_copy(wot_hbm.at[:, pl.ds(pl.multiple_of(h * 256, 256), 256)], wo_ref.at[h], sem_wo.at[h])

        def cp_moe():
            return [pltpu.make_async_copy(wg_hbm, wg_ref, sem_m.at[0]),
                    pltpu.make_async_copy(wu_hbm, wu_ref, sem_m.at[1]),
                    pltpu.make_async_copy(wdt_hbm, wdt_ref, sem_m.at[2])]

        def cp_out(ib):
            return pltpu.make_async_copy(xs_ref.at[ib], o_hbm.at[:, pl.ds(pl.multiple_of(ib * MQ, MQ), MQ)], sem_o.at[ib])

        def layernorm_block(ib):
            xb = xs_ref[ib]
            x = xb.astype(f32)
            mean = jnp.sum(x, axis=0, keepdims=True) * (1.0 / D)
            xc = x - mean
            var = jnp.sum(xc * xc, axis=0, keepdims=True) * (1.0 / D)
            m = _rb(mean)
            v = _rb(var)
            d = _rb(x - m)
            den = _rb(jnp.sqrt(_rb(v + 1e-5)))
            xn = _rb(d / den)
            xnp = jnp.concatenate([xn, jnp.zeros((DP - D, MQ), f32)], axis=0)
            xn_ref[ib] = xnp.T.astype(bf16)
            wrb = wrb_ref[...]
            rs = []
            for j in range(NTQ):
                xj = xn[:, j * 128:(j + 1) * 128]
                bt_ref[ib * NTQ + j] = xj
                acc_ref[ib * NTQ + j] = jnp.zeros((D, 128), f32)
                rs.append(jnp.sum(xj * wrb, axis=0, keepdims=True))
            r_ref[ib] = _rb(jnp.concatenate(rs, axis=1))

        def qproj(ib, hh):
            xn = xn_ref[ib][:, :D]
            q = jnp.dot(xn, wq_ref[hh], preferred_element_type=f32) * QSCALE
            q = q.astype(bf16)
            q_ref[0] = _pk(q[:, :DH])
            q_ref[1] = _pk(q[:, DH:])

        def oproj(ib, hh):
            upd = jnp.dot(wo_ref[hh], jnp.concatenate([_upk(oc_ref[n]) for n in range(NTQ)], axis=1),
                          preferred_element_type=f32)
            for n in range(NTQ):
                acc_ref[ib * NTQ + n] = acc_ref[ib * NTQ + n] + upd[:, n * 128:(n + 1) * 128]

        def epilogue(ib):
            s = _rb(jnp.concatenate([acc_ref[ib * NTQ + j] for j in range(NTQ)], axis=1))
            b = jnp.concatenate([bt_ref[ib * NTQ + j] for j in range(NTQ)], axis=1)
            g = _rb(b * _rb(jax.nn.sigmoid(b)))
            x = xs_ref[ib].astype(f32)
            xs_ref[ib] = (x + _rb(s * g)).astype(bf16)
            cp_out(ib).start()

        def moe():
            for cp in cp_moe():
                cp.wait()
            r = jnp.concatenate([r_ref[j] for j in range(NQ)], axis=0)
            ids = (lax.broadcasted_iota(jnp.int32, (NQ, MQ), 0) * MQ
                   + lax.broadcasted_iota(jnp.int32, (NQ, MQ), 1))
            rows = []
            sel = []
            sub = lax.broadcasted_iota(jnp.int32, (16, DP), 0)
            for c in range(C):
                mx = jnp.max(jnp.max(r, axis=1, keepdims=True), axis=0, keepdims=True)
                idx = jnp.where(r == mx, ids, S)
                idx = jnp.min(jnp.min(idx, axis=1, keepdims=True), axis=0, keepdims=True)
                r = jnp.where(ids == idx, -jnp.inf, r)
                idx_s = jnp.clip(idx[0, 0], 0, S - 1)
                ib = idx_s // MQ
                off = idx_s - ib * MQ
                base = pl.multiple_of((off // 16) * 16, 16)
                blk = xn_ref[ib, pl.ds(base, 16), :].astype(f32)
                row = jnp.sum(jnp.where(sub == off - base, blk, 0.0), axis=0, keepdims=True)
                rows.append(row)
                sel.append((idx_s, mx))
            xsel = jnp.concatenate(rows + rows, axis=0)
            xs16 = xsel[:, :D].astype(bf16)
            g = _rb(jnp.dot(xs16, wg_ref[...], preferred_element_type=f32))
            u = _rb(jnp.dot(xs16, wu_ref[...], preferred_element_type=f32))
            g = _rb(g * _rb(jax.nn.sigmoid(g)))
            hh = (g * u).astype(bf16)
            y = _rb(lax.dot_general(hh, wdt_ref[...], NT, preferred_element_type=f32))
            ypad = jnp.concatenate([y, jnp.zeros((16, DP - D), f32)], axis=1)
            ypad = jnp.concatenate([ypad, jnp.zeros((128 - 16, DP), f32)], axis=0)
            yt = ypad.T[:D]
            lane = lax.broadcasted_iota(jnp.int32, (D, 128), 1)
            for c in range(C):
                idx_s, mx = sel[c]
                yc = _rb(yt[:, c:c + 1] * _rb(jax.nn.sigmoid(mx)))
                tt = idx_s // 128
                old = bt_ref[tt]
                bt_ref[tt] = jnp.where(lane == idx_s - tt * 128, _rb(old + yc), old)

        cp_x(0).start()
        cp_wq(0).start()
        cp_v(0).start()
        cp_k(0).start()
        for ib in range(1, NQ):
            cp_x(ib).start()
        cp_v(1).start()
        cp_wo(0).start()
        cp_wq(1).start()
        z_ref[0] = 0
        oc_ref[...] = jnp.zeros(oc_ref.shape, u32)
        wr = wr_ref[...].astype(f32).reshape(1, D)
        wr = jnp.concatenate([wr, jnp.zeros((1, DP - D), f32)], axis=1)
        wrb_ref[...] = jnp.broadcast_to(wr, (128, DP)).T[:D]
        cp_x(0).wait()
        layernorm_block(0)
        cp_v(0).wait()
        for j in range(NKT):
            vt_ref[0, j] = _pk(v_ref[0, j * 128:(j + 1) * 128, :].T)
        cp_wq(0).wait()
        qproj(0, 0)

        def main_block(t, carry):
            h = t // NQ
            i = t % NQ
            tn = jnp.minimum(t + 1, T - 1)
            i_next = tn % NQ
            h_next = tn // NQ
            tp = jnp.maximum(t - 1, 0)
            i_prev = tp % NQ
            h_prev = tp // NQ
            hv = jnp.minimum(h + 1, HKV - 1)
            z = z_ref[0]
            cur = h % 2
            st = {}

            def qk(name, s_ref, col):
                q = _upk(q_ref[col])
                m = None
                for j in range(S // KBQ):
                    ks = slice(j * KBQ, (j + 1) * KBQ)
                    s = lax.dot_general(k_ref[h, ks, :], q, NT, preferred_element_type=f32)
                    for n in range(NTQ):
                        s_ref[n, ks, :] = s[:, n * 128:(n + 1) * 128]
                    mj = jnp.max(s.reshape(KBQ // 8, 8, MQ), axis=0)
                    m = mj if m is None else jnp.maximum(m, mj)
                st[name] = jnp.max(m, axis=0, keepdims=True)

            def pv(name, s_ref, col):
                acc = None
                m = st[name]
                if gate and name == "a":
                    m = m + jnp.minimum(jnp.abs(st["b"]), 0.0)
                l = None
                for j in range(S // KBP):
                    kd = pl.ds(pl.multiple_of(z + j * KBP, KBP), KBP)
                    sv = jnp.concatenate([s_ref[n, kd, :] for n in range(NTQ)], axis=1)
                    p = jnp.exp2(sv - m)
                    lj = _tree(p, jnp.add)
                    l = lj if l is None else l + lj
                    pb = p.astype(bf16)
                    vt = jnp.concatenate([_upk(vt_ref[cur, jj]) for jj in range(j * KBP // 128, (j + 1) * KBP // 128)], axis=1)
                    oj = jnp.dot(vt, pb, preferred_element_type=f32)
                    acc = oj if acc is None else acc + oj
                l = jnp.sum(l, axis=0, keepdims=True)
                ob = (acc * (1.0 / l)).astype(bf16)
                for n in range(NTQ):
                    oc_ref[n, col * DH // 2:(col + 1) * DH // 2, :] = _pk(ob[:, n * 128:(n + 1) * 128])

            def vtrans():
                for jj in range(VP // 128):
                    off = pl.multiple_of(i * VP + jj * 128, 128)
                    vt_ref[1 - cur, i * (VP // 128) + jj] = _pk(v_ref[hv, pl.ds(off, 128), :].T)

            for o in order.split(","):
                if o == "qa": qk("a", sa_ref, 0)
                elif o == "qb": qk("b", sb_ref, 1)
                elif o == "pa": pv("a", sa_ref, 0)
                elif o == "pb": pv("b", sb_ref, 1)
                elif o == "op": oproj(i_prev, h_prev)
                elif o == "qp": qproj(i_next, h_next)
                elif o == "vt": vtrans()
            return carry

        NSEG = NQ + (HKV - 2) + (NQ - 1)

        def segment(sg, carry):
            mid = sg - (NQ - 1)
            last = sg - (NQ + HKV - 2)
            t0 = jnp.where(sg < NQ, sg, jnp.where(last < 0, mid * NQ, jnp.where(last == 0, T - NQ, T - NQ + 1 + last)))
            n = jnp.where(sg < NQ, 1, jnp.where(last < 0, NQ, jnp.where(last == 0, 2, 1)))
            h = t0 // NQ

            @pl.when(t0 % NQ == 0)
            def _():
                cp_k(h).wait()
                cp_wo(h).wait()

                @pl.when(h + 1 < HKV)
                def _():
                    cp_v(h + 1).wait()
                    cp_wq(h + 1).wait()
                    cp_k(h + 1).start()
                    cp_wo(h + 1).start()

                @pl.when(h + 2 < HKV)
                def _():
                    cp_v(h + 2).start()
                    cp_wq(h + 2).start()

            @pl.when(t0 == MOE_DMA_T)
            def _():
                for cp in cp_moe():
                    cp.start()

            @pl.when(t0 < NQ - 1)
            def _():
                cp_x(t0 + 1).wait()
                layernorm_block(t0 + 1)

            @pl.when(t0 == MOE_T)
            def _():
                moe()

            @pl.when(last > 0)
            def _():
                epilogue(last - 1)

            lax.fori_loop(t0, t0 + n, main_block, 0)
            return carry

        lax.fori_loop(0, NSEG, segment, 0)
        epilogue(NQ - 2)
        oproj(NQ - 1, HKV - 1)
        epilogue(NQ - 1)
        for ib in range(NQ):
            cp_out(ib).wait()

    def fn(A_x, A_k_cache, A_v_cache, A_wq, A_wo, B_x, B_w_r, B_w_gate, B_w_up, B_w_down):
        xt = A_x.reshape(S, D).T
        anyspec = pl.BlockSpec(memory_space=pl.ANY)
        out = pl.pallas_call(
            kernel,
            in_specs=[anyspec, anyspec, anyspec, anyspec, anyspec,
                      pl.BlockSpec(memory_space=pltpu.VMEM),
                      anyspec, anyspec, anyspec],
            out_specs=anyspec,
            out_shape=jax.ShapeDtypeStruct((D, S), bf16),
            scratch_shapes=[
                pltpu.VMEM((NQ, MQ, DP), bf16),
                pltpu.VMEM((NL, D, 128), f32),
                pltpu.VMEM((HKV, S, DH), bf16),
                pltpu.VMEM((HKV, S, DH), bf16),
                pltpu.VMEM((HKV, D, 2 * DH), bf16),
                pltpu.VMEM((HKV, D, 2 * DH), bf16),
                pltpu.VMEM((NTQ, S, 128), f32),
                pltpu.VMEM((NTQ, S, 128), f32),
                pltpu.VMEM((2, MQ // 2, DH), u32),
                pltpu.VMEM((NTQ, DH, 128), u32),
                pltpu.VMEM((2, NKT, DH // 2, 128), u32),
                pltpu.VMEM((NL, D, 128), f32),
                pltpu.VMEM((NQ, D, MQ), bf16),
                pltpu.VMEM((NQ, 1, MQ), f32),
                pltpu.VMEM((D, 128), f32),
                pltpu.VMEM((D, F), bf16),
                pltpu.VMEM((D, F), bf16),
                pltpu.VMEM((D, F), bf16),
                pltpu.SMEM((1,), jnp.int32),
                pltpu.SemaphoreType.DMA((NQ,)),
                pltpu.SemaphoreType.DMA((HKV,)),
                pltpu.SemaphoreType.DMA((HKV,)),
                pltpu.SemaphoreType.DMA((HKV,)),
                pltpu.SemaphoreType.DMA((HKV,)),
                pltpu.SemaphoreType.DMA((3,)),
                pltpu.SemaphoreType.DMA((NQ,)),
            ],
            compiler_params=pltpu.CompilerParams(
                vmem_limit_bytes=VL * 1024 * 1024),
            name="fused_attn_moe",
        )(xt, A_k_cache, A_v_cache, A_wq, A_wo.T, B_w_r, B_w_gate, B_w_up, B_w_down.T)
        return out.T.reshape(1, S, D)

    return fn


_fn = make_kernel()


@jax.jit
def pallas_recurrent_scan__gqa_block_cached__moe_arch_mod__prompt_kernel(
    A_x, A_k_cache, A_v_cache, A_wq, A_wo, B_x, B_w_r, B_w_gate, B_w_up, B_w_down):
    return _fn(A_x, A_k_cache, A_v_cache, A_wq, A_wo, B_x, B_w_r, B_w_gate, B_w_up, B_w_down)
```

```python
import functools
import jax
import jax.numpy as jnp
from jax import lax
import jax.experimental.pallas as pl
import jax.experimental.pallas.tpu as pltpu

S = 2048
D = 576
DP = 640
HQ = 32
HKV = 16
DH = 128
F = 4608
C = 8
LOG2E = 1.4426950408889634
QSCALE = (DH ** -0.5) * LOG2E
bf16 = jnp.bfloat16
f32 = jnp.float32
u32 = jnp.uint32
NT = (((1,), (1,)), ((), ()))


def _rb(x):
    return x.astype(bf16).astype(f32)


def _pk(x):
    return pltpu.bitcast(x, u32)


def _upk(x):
    return pltpu.bitcast(x, bf16)


def _sigmoid(x):
    return 0.5 * jnp.tanh(0.5 * x) + 0.5


def _silu(x):
    h = 0.5 * x
    return h * jnp.tanh(h) + h


def _lin(p, op, n=2):
    parts = [p[i * 8:(i + 1) * 8] for i in range(p.shape[0] // 8)]
    acc = parts[:n]
    for i in range(n, len(parts)):
        acc[i % n] = op(acc[i % n], parts[i])
    while len(acc) > 1:
        acc = [op(acc[i], acc[i + 1]) for i in range(0, len(acc), 2)]
    return acc[0]


def _tree(p, op):
    parts = [p[i * 8:(i + 1) * 8] for i in range(p.shape[0] // 8)]
    while len(parts) > 1:
        nxt = [op(parts[i], parts[i + 1]) for i in range(0, len(parts) - 1, 2)]
        if len(parts) % 2:
            nxt.append(parts[-1])
        parts = nxt
    return parts[0]


def make_kernel(MQ=512, KBQ=2048, KBP=256, VL=110, order="qa,qb,op,pa,qp,pb,vt", MOE_T=12, lag=3, pro=4, H_EARLY=3, moe_dma_seg=4, bulk_seg=1, waitall=False):
    NQ = S // MQ
    NL = S // 128
    NTQ = MQ // 128
    T = HKV * NQ
    VP = S // NQ
    NKT = S // 128

    def kernel(xt_hbm, k_hbm, v_hbm, wq_hbm, wot_hbm, wr_ref, wg_hbm, wu_hbm, wdt_hbm,
               o_hbm,
               xn_ref, acc_ref, k_ref, v_ref, wq_ref, wo_ref,
               sa_ref, sb_ref, q_ref, oc_ref, vt_ref,
               g_ref, xs_ref, r_ref, wrow_ref, wg_ref, wu_ref, wdt_ref, z_ref,
               sem_x, sem_k, sem_v, sem_wq, sem_wo, sem_m, sem_o):

        def cp_x(ib):
            return pltpu.make_async_copy(xt_hbm.at[:, pl.ds(ib * MQ, MQ)], xs_ref.at[ib], sem_x.at[ib])

        def cp_k(h):
            return pltpu.make_async_copy(k_hbm.at[0, h], k_ref.at[h], sem_k.at[h])

        def cp_v(h):
            return pltpu.make_async_copy(v_hbm.at[0, h], v_ref.at[h], sem_v.at[h])

        def cp_wq(h):
            return pltpu.make_async_copy(wq_hbm.at[:, pl.ds(h * 256, 256)], wq_ref.at[h], sem_wq.at[h])

        def cp_wo(h):
            return pltpu.make_async_copy(wot_hbm.at[:, pl.ds(h * 256, 256)], wo_ref.at[h], sem_wo.at[h])

        def cp_moe():
            return [pltpu.make_async_copy(wg_hbm, wg_ref, sem_m.at[0]),
                    pltpu.make_async_copy(wu_hbm, wu_ref, sem_m.at[1]),
                    pltpu.make_async_copy(wdt_hbm, wdt_ref, sem_m.at[2])]

        def cp_out(ib):
            return pltpu.make_async_copy(xs_ref.at[ib], o_hbm.at[:, pl.ds(pl.multiple_of(ib * MQ, MQ), MQ)], sem_o.at[ib])

        def group(h):
            cps = [cp_k(h), cp_wo(h)]
            if h + 1 < HKV:
                cps += [cp_v(h + 1), cp_wq(h + 1)]
            return cps

        def layernorm_block(ib):
            wrow = wrow_ref[...]
            rs = []
            rows = []
            for j in range(NTQ):
                x = xs_ref[ib, :, j * 128:(j + 1) * 128].astype(f32)
                mean = jnp.sum(_lin(x, jnp.add), axis=0, keepdims=True) * (1.0 / D)
                xc = x - mean
                var = jnp.sum(_lin(xc * xc, jnp.add), axis=0, keepdims=True) * (1.0 / D)
                m = _rb(mean)
                inv = 1.0 / _rb(jnp.sqrt(_rb(_rb(var) + 1e-5)))
                xn = (x - m) * inv
                g_ref[ib * NTQ + j] = _silu(xn)
                xnp = jnp.concatenate([xn, jnp.zeros((DP - D, 128), f32)], axis=0).astype(bf16)
                rs.append(jnp.dot(wrow, xnp, preferred_element_type=f32)[0:1, :])
                rows.append(xnp.T)
            xn_ref[ib] = jnp.concatenate(rows, axis=0)
            r_ref[ib] = _rb(jnp.concatenate(rs, axis=1))

        def qproj(ib, hh):
            xn = xn_ref[ib][:, :D]
            q = jnp.dot(xn, wq_ref[hh], preferred_element_type=f32) * QSCALE
            q = q.astype(bf16)
            q_ref[0] = _pk(q[:, :DH])
            q_ref[1] = _pk(q[:, DH:])

        def oproj(ib, hh, jobs=None):
            upd = jnp.dot(wo_ref[hh], jnp.concatenate([_upk(oc_ref[n]) for n in range(NTQ)], axis=1),
                          preferred_element_type=f32)
            if jobs is not None:
                jobs.append(upd[D - 1:D, :])
            for n in range(NTQ):
                acc_ref[ib * NTQ + n] = acc_ref[ib * NTQ + n] + upd[:, n * 128:(n + 1) * 128]

        def epilogue(ib):
            for j in range(NTQ):
                x = xs_ref[ib, :, j * 128:(j + 1) * 128].astype(f32)
                xs_ref[ib, :, j * 128:(j + 1) * 128] = (x + acc_ref[ib * NTQ + j] * g_ref[ib * NTQ + j]).astype(bf16)
            cp_out(ib).start()

        def moe():
            for cp in cp_moe():
                cp.wait()
            r = jnp.concatenate([r_ref[j] for j in range(NQ)], axis=0)
            ids = (lax.broadcasted_iota(jnp.int32, (NQ, MQ), 0) * MQ
                   + lax.broadcasted_iota(jnp.int32, (NQ, MQ), 1))
            rb = lax.shift_right_arithmetic(lax.bitcast_convert_type(r + 0.0, jnp.int32), 16)
            mono = jnp.where(rb < 0, -32769 - rb, rb) + 32768
            key = mono * S + (S - 1 - ids)
            keys = []
            for c in range(C):
                mx = jnp.max(jnp.max(key, axis=1, keepdims=True), axis=0, keepdims=True)
                key = jnp.where(key == mx, -1, key)
                keys.append(mx)
            rows = []
            sel = []
            sub = lax.broadcasted_iota(jnp.int32, (16, DP), 0)
            for c in range(C):
                idx_s = jnp.clip(S - 1 - keys[c][0, 0] % S, 0, S - 1)
                ib = idx_s // MQ
                off = idx_s - ib * MQ
                base = pl.multiple_of((off // 16) * 16, 16)
                blk = xn_ref[ib, pl.ds(base, 16), :].astype(f32)
                rows.append(jnp.sum(jnp.where(sub == off - base, blk, 0.0), axis=0, keepdims=True))
                sel.append(idx_s)
            kv = jnp.concatenate(keys, axis=0)
            mono_s = kv // S - 32768
            rb_s = jnp.where(mono_s < 0, -32769 - mono_s, mono_s)
            rsel = lax.bitcast_convert_type(lax.shift_left(rb_s, 16), f32)
            xsel = jnp.concatenate(rows, axis=0)
            xs16 = jnp.concatenate([xsel, xsel], axis=0)[:, :D].astype(bf16)
            gt = _rb(jnp.dot(xs16, wg_ref[...], preferred_element_type=f32))
            u = _rb(jnp.dot(xs16, wu_ref[...], preferred_element_type=f32))
            hh = (_rb(_silu(gt)) * u).astype(bf16)
            y = _rb(lax.dot_general(hh, wdt_ref[...], NT, preferred_element_type=f32))[:C]
            y = _rb(y * _rb(_sigmoid(rsel)))
            gsel = _silu(_rb(xsel[:, :D] + y))
            gpad = jnp.concatenate([gsel, jnp.zeros((C, DP - D), f32)], axis=1)
            gpad = jnp.concatenate([gpad, jnp.zeros((128 - C, DP), f32)], axis=0)
            gt_all = gpad.T[:D]
            lane = lax.broadcasted_iota(jnp.int32, (D, 128), 1)
            for c in range(C):
                idx_s = sel[c]
                tt = idx_s // 128
                g_ref[tt] = jnp.where(lane == idx_s - tt * 128, gt_all[:, c:c + 1], g_ref[tt])

        w1 = [cp_x(0), cp_v(0), cp_wq(0)]
        w2 = [cp_x(1), cp_k(0), cp_v(1), cp_wo(0)]
        w3 = [cp_wq(1)] + [cp_x(ib) for ib in range(2, NQ)]
        if pro == 1:
            first, second, third = w1 + w2 + w3, [], []
        elif pro == 2:
            first, second, third = w1, w2, w3
        elif pro == 3:
            first, second, third = w1, w2 + w3, []
        elif pro == 4:
            first, second, third = w1 + w2, [], w3
        elif pro == 5:
            first, second, third = w1[:1], w1[1:] + w2, w3
        for cp in first:
            cp.start()
        z_ref[0] = 0
        oc_ref[...] = jnp.zeros(oc_ref.shape, u32)

        def zero_acc(j, c):
            acc_ref[j] = jnp.zeros((D, 128), f32)
            return c
        lax.fori_loop(0, NL, zero_acc, 0)
        wr = wr_ref[...].reshape(1, D)
        wr = jnp.concatenate([wr, jnp.zeros((1, DP - D), bf16)], axis=1)
        wrow_ref[...] = jnp.broadcast_to(wr.astype(f32), (16, DP)).astype(bf16)
        cp_x(0).wait()
        for cp in second:
            cp.start()
        if waitall:
            cp_v(0).wait()
            cp_wq(0).wait()
        layernorm_block(0)
        if not waitall:
            cp_v(0).wait()
        for j in range(NKT):
            vt_ref[0, j] = _pk(v_ref[0, j * 128:(j + 1) * 128, :].T)
        if not waitall:
            cp_wq(0).wait()
        qproj(0, 0)
        for cp in third:
            cp.start()
        for h in range(1, H_EARLY):
            for cp in group(h):
                cp.start()

        def main_block(t, carry):
            h = t // NQ
            i = t % NQ
            tn = jnp.minimum(t + 1, T - 1)
            i_next = tn % NQ
            h_next = tn // NQ
            tp = jnp.maximum(t - 1, 0)
            i_prev = tp % NQ
            h_prev = tp // NQ
            hv = jnp.minimum(h + 1, HKV - 1)
            z = z_ref[0]
            cur = h % 2
            st = {}
            jobs = []

            def qk(name, s_ref, col):
                q = _upk(q_ref[col])
                m = None
                for j in range(S // KBQ):
                    ks = slice(j * KBQ, (j + 1) * KBQ)
                    s = lax.dot_general(k_ref[h, ks, :], q, NT, preferred_element_type=f32)
                    for n in range(NTQ):
                        s_ref[n, ks, :] = s[:, n * 128:(n + 1) * 128]
                    mj = jnp.max(s.reshape(KBQ // 8, 8, MQ), axis=0)
                    m = mj if m is None else jnp.maximum(m, mj)
                st[name] = jnp.max(m, axis=0, keepdims=True)
                jobs.append(st[name])

            def pv(name, s_ref, col):
                acc = None
                m = st[name]
                if name == "a":
                    m = m + jnp.minimum(jnp.abs(st["b"]), 0.0)
                l = None
                for j in range(S // KBP):
                    kd = pl.ds(pl.multiple_of(z + j * KBP, KBP), KBP)
                    sv = jnp.concatenate([s_ref[n, kd, :] for n in range(NTQ)], axis=1)
                    mg = m
                    if lag and len(jobs) >= lag:
                        mg = m + jnp.minimum(jnp.abs(jobs[-lag]), 0.0)
                    p = jnp.exp2(sv - mg)
                    lj = _tree(p, jnp.add)
                    l = lj if l is None else l + lj
                    pb = p.astype(bf16)
                    vt = jnp.concatenate([_upk(vt_ref[cur, jj]) for jj in range(j * KBP // 128, (j + 1) * KBP // 128)], axis=1)
                    oj = jnp.dot(vt, pb, preferred_element_type=f32)
                    jobs.append(oj[DH - 1:DH, :])
                    acc = oj if acc is None else acc + oj
                l = jnp.sum(l, axis=0, keepdims=True)
                ob = (acc * (1.0 / l)).astype(bf16)
                for n in range(NTQ):
                    oc_ref[n, col * DH // 2:(col + 1) * DH // 2, :] = _pk(ob[:, n * 128:(n + 1) * 128])

            def vtrans():
                for jj in range(VP // 128):
                    off = pl.multiple_of(i * VP + jj * 128, 128)
                    vt_ref[1 - cur, i * (VP // 128) + jj] = _pk(v_ref[hv, pl.ds(off, 128), :].T)

            for o in order.split(","):
                if o == "qa": qk("a", sa_ref, 0)
                elif o == "qb": qk("b", sb_ref, 1)
                elif o == "pa": pv("a", sa_ref, 0)
                elif o == "pb": pv("b", sb_ref, 1)
                elif o == "op": oproj(i_prev, h_prev, jobs)
                elif o == "qp": qproj(i_next, h_next)
                elif o == "vt": vtrans()
            return carry

        def pair_block(p, carry):
            main_block(2 * p, carry)
            main_block(2 * p + 1, carry)
            return carry

        starts = [0, 1, 2, 3] + [h * NQ for h in range(1, H_EARLY)] + [MOE_T, T - 2, T - 1, T]
        assert MOE_T == H_EARLY * NQ
        NSEG = len(starts) - 1
        SEG_MOE = NSEG - 3

        def segment(sg, carry):
            t0 = jnp.int32(0)
            t1 = jnp.int32(0)
            for k in range(NSEG):
                t0 = jnp.where(sg == k, starts[k], t0)
                t1 = jnp.where(sg == k, starts[k + 1], t1)
            paired = jnp.logical_and(sg >= NQ, sg <= SEG_MOE)

            @pl.when(sg < NQ - 1)
            def _():
                cp_x(sg + 1).wait()
                layernorm_block(sg + 1)

            @pl.when(sg == 0)
            def _():
                cp_k(0).wait()
                cp_v(1).wait()
                cp_wo(0).wait()

            @pl.when(sg == NQ - 1)
            def _():
                cp_wq(1).wait()

            if bulk_seg >= 0:
                @pl.when(sg == bulk_seg)
                def _():
                    for h in range(H_EARLY, HKV):
                        for cp in group(h):
                            cp.start()

            if moe_dma_seg >= 0:
                @pl.when(sg == moe_dma_seg)
                def _():
                    for cp in cp_moe():
                        cp.start()

            for h in range(1, H_EARLY):
                @pl.when(sg == NQ - 1 + h)
                def _(h=h):
                    for cp in group(h):
                        cp.wait()

            @pl.when(sg == SEG_MOE)
            def _():
                for h in range(H_EARLY, HKV):
                    for cp in group(h):
                        cp.wait()
                moe()

            @pl.when(sg >= NSEG - 2)
            def _():
                epilogue(sg - (NSEG - 2))

            p0 = jnp.where(paired, t0 // 2, 0)
            p1 = jnp.where(paired, t1 // 2, 0)
            lax.fori_loop(p0, p1, pair_block, 0)
            lax.fori_loop(jnp.where(paired, 0, t0), jnp.where(paired, 0, t1), main_block, 0)
            return carry

        lax.fori_loop(0, NSEG, segment, 0)
        epilogue(NQ - 2)
        oproj(NQ - 1, HKV - 1)
        epilogue(NQ - 1)
        for ib in range(NQ):
            cp_out(ib).wait()

    def fn(A_x, A_k_cache, A_v_cache, A_wq, A_wo, B_x, B_w_r, B_w_gate, B_w_up, B_w_down):
        xt = A_x.reshape(S, D).T
        anyspec = pl.BlockSpec(memory_space=pl.ANY)
        out = pl.pallas_call(
            kernel,
            in_specs=[anyspec, anyspec, anyspec, anyspec, anyspec,
                      pl.BlockSpec(memory_space=pltpu.VMEM),
                      anyspec, anyspec, anyspec],
            out_specs=anyspec,
            out_shape=jax.ShapeDtypeStruct((D, S), bf16),
            scratch_shapes=[
                pltpu.VMEM((NQ, MQ, DP), bf16),
                pltpu.VMEM((NL, D, 128), f32),
                pltpu.VMEM((HKV, S, DH), bf16),
                pltpu.VMEM((HKV, S, DH), bf16),
                pltpu.VMEM((HKV, D, 2 * DH), bf16),
                pltpu.VMEM((HKV, D, 2 * DH), bf16),
                pltpu.VMEM((NTQ, S, 128), f32),
                pltpu.VMEM((NTQ, S, 128), f32),
                pltpu.VMEM((2, MQ // 2, DH), u32),
                pltpu.VMEM((NTQ, DH, 128), u32),
                pltpu.VMEM((2, NKT, DH // 2, 128), u32),
                pltpu.VMEM((NL, D, 128), f32),
                pltpu.VMEM((NQ, D, MQ), bf16),
                pltpu.VMEM((NQ, 1, MQ), f32),
                pltpu.VMEM((16, DP), bf16),
                pltpu.VMEM((D, F), bf16),
                pltpu.VMEM((D, F), bf16),
                pltpu.VMEM((D, F), bf16),
                pltpu.SMEM((1,), jnp.int32),
                pltpu.SemaphoreType.DMA((NQ,)),
                pltpu.SemaphoreType.DMA((HKV,)),
                pltpu.SemaphoreType.DMA((HKV,)),
                pltpu.SemaphoreType.DMA((HKV,)),
                pltpu.SemaphoreType.DMA((HKV,)),
                pltpu.SemaphoreType.DMA((3,)),
                pltpu.SemaphoreType.DMA((NQ,)),
            ],
            compiler_params=pltpu.CompilerParams(
                vmem_limit_bytes=VL * 1024 * 1024),
            name="fused_attn_moe",
        )(xt, A_k_cache, A_v_cache, A_wq, A_wo.T, B_w_r, B_w_gate, B_w_up, B_w_down.T)
        return out.T.reshape(1, S, D)

    return fn


_fn = make_kernel()


@jax.jit
def pallas_recurrent_scan__gqa_block_cached__moe_arch_mod__prompt_kernel(
    A_x, A_k_cache, A_v_cache, A_wq, A_wo, B_x, B_w_r, B_w_gate, B_w_up, B_w_down):
    return _fn(A_x, A_k_cache, A_v_cache, A_wq, A_wo, B_x, B_w_r, B_w_gate, B_w_up, B_w_down)
```

```python
import functools
import jax
import jax.numpy as jnp
from jax import lax
import jax.experimental.pallas as pl
import jax.experimental.pallas.tpu as pltpu

S = 2048
D = 576
DP = 640
HQ = 32
HKV = 16
DH = 128
F = 4608
C = 8
LOG2E = 1.4426950408889634
QSCALE = (DH ** -0.5) * LOG2E
bf16 = jnp.bfloat16
f32 = jnp.float32
u32 = jnp.uint32
NT = (((1,), (1,)), ((), ()))


def _rb(x):
    return x.astype(bf16).astype(f32)


def _pk(x):
    return pltpu.bitcast(x, u32)


def _upk(x):
    return pltpu.bitcast(x, bf16)


def _sigmoid(x):
    return 0.5 * jnp.tanh(0.5 * x) + 0.5


def _silu(x):
    h = 0.5 * x
    return h * jnp.tanh(h) + h


def _lin(p, op, n=2):
    parts = [p[i * 8:(i + 1) * 8] for i in range(p.shape[0] // 8)]
    acc = parts[:n]
    for i in range(n, len(parts)):
        acc[i % n] = op(acc[i % n], parts[i])
    while len(acc) > 1:
        acc = [op(acc[i], acc[i + 1]) for i in range(0, len(acc), 2)]
    return acc[0]


def _tree(p, op):
    parts = [p[i * 8:(i + 1) * 8] for i in range(p.shape[0] // 8)]
    while len(parts) > 1:
        nxt = [op(parts[i], parts[i + 1]) for i in range(0, len(parts) - 1, 2)]
        if len(parts) % 2:
            nxt.append(parts[-1])
        parts = nxt
    return parts[0]


def make_kernel(MQ=512, KBQ=2048, KBP=128, VL=110, order="qa,qb,op,pa,qp,pb,vt", MOE_T=12, lag=5, pro=4, H_EARLY=3, moe_dma_seg=4, bulk_seg=1, waitall=True, topk_filler=True, split=2, mstore=True, U=2, late=False, ln1=1, rc=4):
    NQ = S // MQ
    NL = S // 128
    NTQ = MQ // 128
    T = HKV * NQ
    VP = S // NQ
    NKT = S // 128

    def kernel(xt_hbm, k_hbm, v_hbm, wq_hbm, wot_hbm, wr_ref, wg_hbm, wu_hbm, wdt_hbm,
               o_hbm,
               xn_ref, acc_ref, k_ref, v_ref, wq_ref, wo_ref,
               sa_ref, sb_ref, q_ref, oc_ref, vt_ref,
               g_ref, xs_ref, r_ref, wrow_ref, wg_ref, wu_ref, wdt_ref, rsel_ref, z_ref, idx_ref,
               sem_x, sem_k, sem_v, sem_wq, sem_wo, sem_m, sem_o, sem_t):

        def cp_x(ib):
            return pltpu.make_async_copy(xt_hbm.at[:, pl.ds(ib * MQ, MQ)], xs_ref.at[ib], sem_x.at[ib])

        def cp_k(h):
            return pltpu.make_async_copy(k_hbm.at[0, h], k_ref.at[h], sem_k.at[h])

        def cp_v(h):
            return pltpu.make_async_copy(v_hbm.at[0, h], v_ref.at[h], sem_v.at[h])

        def cp_wq(h):
            return pltpu.make_async_copy(wq_hbm.at[:, pl.ds(h * 256, 256)], wq_ref.at[h], sem_wq.at[h])

        def cp_wo(h):
            return pltpu.make_async_copy(wot_hbm.at[:, pl.ds(h * 256, 256)], wo_ref.at[h], sem_wo.at[h])

        def cp_moe():
            return [pltpu.make_async_copy(wg_hbm, wg_ref, sem_m.at[0]),
                    pltpu.make_async_copy(wu_hbm, wu_ref, sem_m.at[1]),
                    pltpu.make_async_copy(wdt_hbm, wdt_ref, sem_m.at[2])]

        def cp_out(ib):
            return pltpu.make_async_copy(xs_ref.at[ib], o_hbm.at[:, pl.ds(pl.multiple_of(ib * MQ, MQ), MQ)], sem_o.at[ib])

        def group(h):
            cps = [cp_k(h), cp_wo(h)]
            if h + 1 < HKV:
                cps += [cp_v(h + 1), cp_wq(h + 1)]
            return cps

        def layernorm_tiles(ib, tiles):
            wrow = wrow_ref[...]
            for j in tiles:
                x = xs_ref[ib, :, j * 128:(j + 1) * 128].astype(f32)
                mean = jnp.sum(_lin(x, jnp.add), axis=0, keepdims=True) * (1.0 / D)
                xc = x - mean
                var = jnp.sum(_lin(xc * xc, jnp.add), axis=0, keepdims=True) * (1.0 / D)
                m = _rb(mean)
                inv = 1.0 / _rb(jnp.sqrt(_rb(_rb(var) + 1e-5)))
                xn = (x - m) * inv
                g_ref[ib * NTQ + j] = _silu(xn)
                xnp = jnp.concatenate([xn, jnp.zeros((DP - D, 128), f32)], axis=0).astype(bf16)
                r_ref[ib, :, j * 128:(j + 1) * 128] = _rb(jnp.dot(wrow, xnp, preferred_element_type=f32)[0:1, :])
                xn_ref[ib, j * 128:(j + 1) * 128, :] = xnp.T

        def layernorm_block(ib):
            layernorm_tiles(ib, range(NTQ))

        def qproj(ib, hh):
            xn = xn_ref[ib][:, :D]
            q = jnp.dot(xn, wq_ref[hh], preferred_element_type=f32) * QSCALE
            q = q.astype(bf16)
            q_ref[0] = _pk(q[:, :DH])
            q_ref[1] = _pk(q[:, DH:])

        def oproj(ib, hh, jobs=None):
            upd = jnp.dot(wo_ref[hh], jnp.concatenate([_upk(oc_ref[n]) for n in range(NTQ)], axis=1),
                          preferred_element_type=f32)
            if jobs is not None:
                jobs.append(upd[D - 1:D, :])
            for n in range(NTQ):
                acc_ref[ib * NTQ + n] = acc_ref[ib * NTQ + n] + upd[:, n * 128:(n + 1) * 128]

        def epilogue(ib):
            for j in range(NTQ):
                x = xs_ref[ib, :, j * 128:(j + 1) * 128].astype(f32)
                xs_ref[ib, :, j * 128:(j + 1) * 128] = (x + acc_ref[ib * NTQ + j] * g_ref[ib * NTQ + j]).astype(bf16)
            cp_out(ib).start()

        def topk():
            r = jnp.concatenate([r_ref[j] for j in range(NQ)], axis=0)
            ids = (lax.broadcasted_iota(jnp.int32, (NQ, MQ), 0) * MQ
                   + lax.broadcasted_iota(jnp.int32, (NQ, MQ), 1))
            rb = lax.shift_right_arithmetic(lax.bitcast_convert_type(r + 0.0, jnp.int32), 16)
            mono = jnp.where(rb < 0, -32769 - rb, rb) + 32768
            key = mono * S + (S - 1 - ids)
            keys = []
            for c in range(C):
                mx = jnp.max(jnp.max(key, axis=1, keepdims=True), axis=0, keepdims=True)
                key = jnp.where(key == mx, -1, key)
                keys.append(mx)
                idx_ref[c] = S - 1 - mx[0, 0] % S
            kv = jnp.concatenate(keys, axis=0)
            mono_s = kv // S - 32768
            rb_s = jnp.where(mono_s < 0, -32769 - mono_s, mono_s)
            rsel_ref[...] = jnp.broadcast_to(lax.bitcast_convert_type(lax.shift_left(rb_s, 16), f32), (C, 128))

        def moe():
            for cp in cp_moe():
                cp.wait()
            rows = []
            sel = []
            sub = lax.broadcasted_iota(jnp.int32, (16, DP), 0)
            for c in range(C):
                idx_s = jnp.clip(idx_ref[c], 0, S - 1)
                ib = idx_s // MQ
                off = idx_s - ib * MQ
                base = pl.multiple_of((off // 16) * 16, 16)
                blk = xn_ref[ib, pl.ds(base, 16), :].astype(f32)
                rows.append(jnp.sum(jnp.where(sub == off - base, blk, 0.0), axis=0, keepdims=True))
                sel.append(idx_s)
            rsel = rsel_ref[:, 0:1]
            xsel = jnp.concatenate(rows, axis=0)
            xs16 = jnp.concatenate([xsel, xsel], axis=0)[:, :D].astype(bf16)
            gt = _rb(jnp.dot(xs16, wg_ref[...], preferred_element_type=f32))
            u = _rb(jnp.dot(xs16, wu_ref[...], preferred_element_type=f32))
            hh = (_rb(_silu(gt)) * u).astype(bf16)
            y = _rb(lax.dot_general(hh, wdt_ref[...], NT, preferred_element_type=f32))[:C]
            y = _rb(y * _rb(_sigmoid(rsel)))
            gsel = _silu(_rb(xsel[:, :D] + y))
            gpad = jnp.concatenate([gsel, jnp.zeros((C, DP - D), f32)], axis=1)
            gpad = jnp.concatenate([gpad, jnp.zeros((128 - C, DP), f32)], axis=0)
            gt_all = gpad.T[:D]
            lane = lax.broadcasted_iota(jnp.int32, (D, 128), 1)
            for c in range(C):
                idx_s = sel[c]
                tt = idx_s // 128
                if mstore:
                    pltpu.store(g_ref.at[tt], jnp.broadcast_to(gt_all[:, c:c + 1], (D, 128)), mask=lane == idx_s - tt * 128)
                else:
                    g_ref[tt] = jnp.where(lane == idx_s - tt * 128, gt_all[:, c:c + 1], g_ref[tt])

        w1 = [cp_x(0), cp_v(0), cp_wq(0)]
        w2 = [cp_x(1), cp_k(0)] + ([] if late else [cp_v(1), cp_wo(0)])
        w3 = ([cp_v(1), cp_wo(0)] if late else []) + [cp_wq(1)] + [cp_x(ib) for ib in range(2, NQ)]
        if pro == 1:
            first, second, third = w1 + w2 + w3, [], []
        elif pro == 2:
            first, second, third = w1, w2, w3
        elif pro == 3:
            first, second, third = w1, w2 + w3, []
        elif pro == 4:
            first, second, third = w1 + w2, [], w3
        elif pro == 5:
            first, second, third = w1[:1], w1[1:] + w2, w3
        for cp in first:
            cp.start()
        z_ref[0] = 0
        r_ref[...] = jnp.zeros(r_ref.shape, f32)
        oc_ref[...] = jnp.zeros(oc_ref.shape, u32)

        def zero_acc(j, c):
            acc_ref[j] = jnp.zeros((D, 128), f32)
            return c
        lax.fori_loop(0, NL, zero_acc, 0)
        wr = wr_ref[...].reshape(1, D)
        wr = jnp.concatenate([wr, jnp.zeros((1, DP - D), bf16)], axis=1)
        wrow_ref[...] = jnp.broadcast_to(wr.astype(f32), (16, DP)).astype(bf16)
        cp_x(0).wait()
        for cp in second:
            cp.start()
        layernorm_tiles(0, range(split))
        cp_v(0).wait()
        if waitall:
            cp_wq(0).wait()
        layernorm_tiles(0, range(split, NTQ))
        for j in range(NKT):
            vt_ref[0, j] = _pk(v_ref[0, j * 128:(j + 1) * 128, :].T)
        if not waitall:
            cp_wq(0).wait()
        if ln1 == 1:
            cp_x(1).wait()
            qproj(0, 0)
            layernorm_block(1)
        elif ln1 == 2:
            cp_x(1).wait()
            layernorm_block(1)
            qproj(0, 0)
        else:
            qproj(0, 0)
        for cp in third:
            cp.start()
        for h in range(1, H_EARLY):
            for cp in group(h):
                cp.start()

        def main_block(t, carry):
            h = t // NQ
            i = t % NQ
            tn = jnp.minimum(t + 1, T - 1)
            i_next = tn % NQ
            h_next = tn // NQ
            tp = jnp.maximum(t - 1, 0)
            i_prev = tp % NQ
            h_prev = tp // NQ
            hv = jnp.minimum(h + 1, HKV - 1)
            z = z_ref[0]
            cur = h % 2
            st = {}
            jobs = []

            def qk(name, s_ref, col):
                q = _upk(q_ref[col])
                m = None
                for j in range(S // KBQ):
                    ks = slice(j * KBQ, (j + 1) * KBQ)
                    s = lax.dot_general(k_ref[h, ks, :], q, NT, preferred_element_type=f32)
                    for n in range(NTQ):
                        s_ref[n, ks, :] = s[:, n * 128:(n + 1) * 128]
                    mj = jnp.max(s.reshape(KBQ // 8, 8, MQ), axis=0)
                    m = mj if m is None else jnp.maximum(m, mj)
                st[name] = jnp.max(m, axis=0, keepdims=True)
                jobs.append(st[name])

            def pv(name, s_ref, col):
                acc = None
                m = st[name]
                if name == "a":
                    m = m + jnp.minimum(jnp.abs(st["b"]), 0.0)
                l = None
                for j in range(S // KBP):
                    kd = pl.ds(pl.multiple_of(z + j * KBP, KBP), KBP)
                    sv = jnp.concatenate([s_ref[n, kd, :] for n in range(NTQ)], axis=1)
                    mg = m
                    if lag and len(jobs) >= lag:
                        mg = m + jnp.minimum(jnp.abs(jobs[-lag]), 0.0)
                    p = jnp.exp2(sv - mg)
                    lj = _tree(p, jnp.add)
                    l = lj if l is None else l + lj
                    pb = p.astype(bf16)
                    vt = jnp.concatenate([_upk(vt_ref[cur, jj]) for jj in range(j * KBP // 128, (j + 1) * KBP // 128)], axis=1)
                    oj = jnp.dot(vt, pb, preferred_element_type=f32)
                    jobs.append(oj[DH - 1:DH, :])
                    acc = oj if acc is None else acc + oj
                l = jnp.sum(l, axis=0, keepdims=True)
                ob = (acc * (1.0 / l)).astype(bf16)
                for n in range(NTQ):
                    oc_ref[n, col * DH // 2:(col + 1) * DH // 2, :] = _pk(ob[:, n * 128:(n + 1) * 128])

            def vtrans():
                for jj in range(VP // 128):
                    off = pl.multiple_of(i * VP + jj * 128, 128)
                    vt_ref[1 - cur, i * (VP // 128) + jj] = _pk(v_ref[hv, pl.ds(off, 128), :].T)

            for o in order.split(","):
                if o == "qa": qk("a", sa_ref, 0)
                elif o == "qb": qk("b", sb_ref, 1)
                elif o == "pa": pv("a", sa_ref, 0)
                elif o == "pb": pv("b", sb_ref, 1)
                elif o == "op": oproj(i_prev, h_prev, jobs)
                elif o == "qp": qproj(i_next, h_next)
                elif o == "vt": vtrans()
            return carry

        def single_block(t, carry):
            if topk_filler:
                topk()
            return main_block(t, carry)

        def multi_block(p, carry):
            for u in range(U):
                main_block(U * p + u, carry)
            return carry

        TM = NQ + ((T - 2 - NQ) // U) * U
        starts = [0, 1, 2, 3] + [h * NQ for h in range(1, H_EARLY)] + [MOE_T, TM, T - 2, T - 1, T]
        assert MOE_T == H_EARLY * NQ
        NSEG = len(starts) - 1
        SEG_MOE = NSEG - 4

        def segment(sg, carry):
            t0 = jnp.int32(0)
            t1 = jnp.int32(0)
            for k in range(NSEG):
                t0 = jnp.where(sg == k, starts[k], t0)
                t1 = jnp.where(sg == k, starts[k + 1], t1)
            paired = jnp.logical_and(sg >= NQ, sg <= SEG_MOE)

            @pl.when(jnp.logical_and(sg < NQ - 1, sg >= (1 if ln1 else 0)))
            def _():
                cp_x(sg + 1).wait()
                layernorm_block(sg + 1)

            @pl.when(sg == 0)
            def _():
                cp_k(0).wait()
                if not late:
                    cp_v(1).wait()
                    cp_wo(0).wait()

            if late:
                @pl.when(sg == 1)
                def _():
                    cp_v(1).wait()
                    cp_wo(0).wait()

            @pl.when(sg == NQ - 1)
            def _():
                cp_wq(1).wait()

            if bulk_seg >= 0:
                @pl.when(sg == bulk_seg)
                def _():
                    for h in range(H_EARLY, HKV):
                        for cp in group(h):
                            cp.start()

            if moe_dma_seg >= 0:
                @pl.when(sg == moe_dma_seg)
                def _():
                    for cp in cp_moe():
                        cp.start()

            for h in range(1, H_EARLY):
                @pl.when(sg == NQ - 1 + h)
                def _(h=h):
                    for cp in group(h):
                        cp.wait()

            @pl.when(sg == SEG_MOE)
            def _():
                for h in range(H_EARLY, HKV):
                    for cp in group(h):
                        cp.wait()
                if not topk_filler:
                    topk()
                moe()

            @pl.when(sg >= NSEG - 2)
            def _():
                epilogue(sg - (NSEG - 2))

            p0 = jnp.where(paired, t0 // U, 0)
            p1 = jnp.where(paired, t1 // U, 0)
            lax.fori_loop(p0, p1, multi_block, 0)
            lax.fori_loop(jnp.where(paired, 0, t0), jnp.where(paired, 0, t1), single_block, 0)
            return carry

        lax.fori_loop(0, NSEG, segment, 0)
        epilogue(NQ - 2)
        if rc:
            ib = NQ - 1
            upd = jnp.dot(wo_ref[HKV - 1], jnp.concatenate([_upk(oc_ref[n]) for n in range(NTQ)], axis=1),
                          preferred_element_type=f32)
            RR = D // rc
            outs = []
            for c in range(rc):
                rows = slice(c * RR, (c + 1) * RR)
                for n in range(NTQ):
                    cols = slice(n * 128, (n + 1) * 128)
                    sv = acc_ref[ib * NTQ + n, rows, :] + upd[rows, cols]
                    x = xs_ref[ib, rows, cols].astype(f32)
                    xs_ref[ib, rows, cols] = (x + sv * g_ref[ib * NTQ + n, rows, :]).astype(bf16)
                cp = pltpu.make_async_copy(xs_ref.at[ib, pl.ds(c * RR, RR)], o_hbm.at[pl.ds(c * RR, RR), pl.ds(ib * MQ, MQ)], sem_t.at[c])
                cp.start()
                outs.append(cp)
            for ib2 in range(NQ - 1):
                cp_out(ib2).wait()
            for cp in outs:
                cp.wait()
        else:
            oproj(NQ - 1, HKV - 1)
            epilogue(NQ - 1)
            for ib in range(NQ):
                cp_out(ib).wait()

    def fn(A_x, A_k_cache, A_v_cache, A_wq, A_wo, B_x, B_w_r, B_w_gate, B_w_up, B_w_down):
        xt = A_x.reshape(S, D).T
        anyspec = pl.BlockSpec(memory_space=pl.ANY)
        out = pl.pallas_call(
            kernel,
            in_specs=[anyspec, anyspec, anyspec, anyspec, anyspec,
                      pl.BlockSpec(memory_space=pltpu.VMEM),
                      anyspec, anyspec, anyspec],
            out_specs=anyspec,
            out_shape=jax.ShapeDtypeStruct((D, S), bf16),
            scratch_shapes=[
                pltpu.VMEM((NQ, MQ, DP), bf16),
                pltpu.VMEM((NL, D, 128), f32),
                pltpu.VMEM((HKV, S, DH), bf16),
                pltpu.VMEM((HKV, S, DH), bf16),
                pltpu.VMEM((HKV, D, 2 * DH), bf16),
                pltpu.VMEM((HKV, D, 2 * DH), bf16),
                pltpu.VMEM((NTQ, S, 128), f32),
                pltpu.VMEM((NTQ, S, 128), f32),
                pltpu.VMEM((2, MQ // 2, DH), u32),
                pltpu.VMEM((NTQ, DH, 128), u32),
                pltpu.VMEM((2, NKT, DH // 2, 128), u32),
                pltpu.VMEM((NL, D, 128), f32),
                pltpu.VMEM((NQ, D, MQ), bf16),
                pltpu.VMEM((NQ, 1, MQ), f32),
                pltpu.VMEM((16, DP), bf16),
                pltpu.VMEM((D, F), bf16),
                pltpu.VMEM((D, F), bf16),
                pltpu.VMEM((D, F), bf16),
                pltpu.VMEM((C, 128), f32),
                pltpu.SMEM((1,), jnp.int32),
                pltpu.SMEM((C,), jnp.int32),
                pltpu.SemaphoreType.DMA((NQ,)),
                pltpu.SemaphoreType.DMA((HKV,)),
                pltpu.SemaphoreType.DMA((HKV,)),
                pltpu.SemaphoreType.DMA((HKV,)),
                pltpu.SemaphoreType.DMA((HKV,)),
                pltpu.SemaphoreType.DMA((3,)),
                pltpu.SemaphoreType.DMA((NQ,)),
                pltpu.SemaphoreType.DMA((4,)),
            ],
            compiler_params=pltpu.CompilerParams(
                vmem_limit_bytes=VL * 1024 * 1024),
            name="fused_attn_moe",
        )(xt, A_k_cache, A_v_cache, A_wq, A_wo.T, B_w_r, B_w_gate, B_w_up, B_w_down.T)
        return out.T.reshape(1, S, D)

    return fn


_fn = make_kernel()


@jax.jit
def pallas_recurrent_scan__gqa_block_cached__moe_arch_mod__prompt_kernel(
    A_x, A_k_cache, A_v_cache, A_wq, A_wo, B_x, B_w_r, B_w_gate, B_w_up, B_w_down):
    return _fn(A_x, A_k_cache, A_v_cache, A_wq, A_wo, B_x, B_w_r, B_w_gate, B_w_up, B_w_down)
```

```python
import functools
import jax
import jax.numpy as jnp
from jax import lax
import jax.experimental.pallas as pl
import jax.experimental.pallas.tpu as pltpu

S = 2048
D = 576
DP = 640
HQ = 32
HKV = 16
DH = 128
F = 4608
C = 8
LOG2E = 1.4426950408889634
QSCALE = (DH ** -0.5) * LOG2E
bf16 = jnp.bfloat16
f32 = jnp.float32
u32 = jnp.uint32
NT = (((1,), (1,)), ((), ()))


def _rb(x):
    return x.astype(bf16).astype(f32)


def _pk(x):
    return pltpu.bitcast(x, u32)


def _upk(x):
    return pltpu.bitcast(x, bf16)


def _sigmoid(x):
    return 0.5 * jnp.tanh(0.5 * x) + 0.5


def _silu(x):
    h = 0.5 * x
    return h * jnp.tanh(h) + h


def _lin(p, op, n=2):
    parts = [p[i * 8:(i + 1) * 8] for i in range(p.shape[0] // 8)]
    acc = parts[:n]
    for i in range(n, len(parts)):
        acc[i % n] = op(acc[i % n], parts[i])
    while len(acc) > 1:
        acc = [op(acc[i], acc[i + 1]) for i in range(0, len(acc), 2)]
    return acc[0]


def _tree(p, op):
    parts = [p[i * 8:(i + 1) * 8] for i in range(p.shape[0] // 8)]
    while len(parts) > 1:
        nxt = [op(parts[i], parts[i + 1]) for i in range(0, len(parts) - 1, 2)]
        if len(parts) % 2:
            nxt.append(parts[-1])
        parts = nxt
    return parts[0]


def make_kernel(MQ=512, KBQ=2048, KBP=128, VL=110, order="qa,qb,op,pa,qp,pb,vt", MOE_T=12, lag=5, pro=4, H_EARLY=3, moe_dma_seg=3, bulk_seg=0, waitall=True, topk_filler=True, split=2, mstore=True, U=2, late=False, ln1=0, rc=4):
    NQ = S // MQ
    NL = S // 128
    NTQ = MQ // 128
    T = HKV * NQ
    VP = S // NQ
    NKT = S // 128

    def kernel(xt_hbm, k_hbm, v_hbm, wq_hbm, wot_hbm, wr_ref, wg_hbm, wu_hbm, wdt_hbm,
               o_hbm,
               xn_ref, acc_ref, k_ref, v_ref, wq_ref, wo_ref,
               sa_ref, sb_ref, q_ref, oc_ref, vt_ref,
               g_ref, xs_ref, r_ref, wrow_ref, wg_ref, wu_ref, wdt_ref, rsel_ref, z_ref, idx_ref,
               sem_x, sem_k, sem_v, sem_wq, sem_wo, sem_m, sem_o, sem_t):

        def cp_x(ib):
            return pltpu.make_async_copy(xt_hbm.at[:, pl.ds(ib * MQ, MQ)], xs_ref.at[ib], sem_x.at[ib])

        def cp_k(h):
            return pltpu.make_async_copy(k_hbm.at[0, h], k_ref.at[h], sem_k.at[h])

        def cp_v(h):
            return pltpu.make_async_copy(v_hbm.at[0, h], v_ref.at[h], sem_v.at[h])

        def cp_wq(h):
            return pltpu.make_async_copy(wq_hbm.at[:, pl.ds(h * 256, 256)], wq_ref.at[h], sem_wq.at[h])

        def cp_wo(h):
            return pltpu.make_async_copy(wot_hbm.at[:, pl.ds(h * 256, 256)], wo_ref.at[h], sem_wo.at[h])

        def cp_moe():
            return [pltpu.make_async_copy(wg_hbm, wg_ref, sem_m.at[0]),
                    pltpu.make_async_copy(wu_hbm, wu_ref, sem_m.at[1]),
                    pltpu.make_async_copy(wdt_hbm, wdt_ref, sem_m.at[2])]

        def cp_out(ib):
            return pltpu.make_async_copy(xs_ref.at[ib], o_hbm.at[:, pl.ds(pl.multiple_of(ib * MQ, MQ), MQ)], sem_o.at[ib])

        def cp_tail(c):
            RR = D // rc
            return pltpu.make_async_copy(xs_ref.at[NQ - 1, pl.ds(c * RR, RR)],
                                         o_hbm.at[pl.ds(c * RR, RR), pl.ds((NQ - 1) * MQ, MQ)], sem_t.at[c])

        def group(h):
            cps = [cp_k(h), cp_wo(h)]
            if h + 1 < HKV:
                cps += [cp_v(h + 1), cp_wq(h + 1)]
            return cps

        def layernorm_tiles(ib, tiles):
            wrow = wrow_ref[...]
            for j in tiles:
                x = xs_ref[ib, :, j * 128:(j + 1) * 128].astype(f32)
                mean = jnp.sum(_lin(x, jnp.add), axis=0, keepdims=True) * (1.0 / D)
                xc = x - mean
                var = jnp.sum(_lin(xc * xc, jnp.add), axis=0, keepdims=True) * (1.0 / D)
                m = _rb(mean)
                inv = 1.0 / _rb(jnp.sqrt(_rb(_rb(var) + 1e-5)))
                xn = (x - m) * inv
                g_ref[ib * NTQ + j] = _silu(xn)
                xnp = jnp.concatenate([xn, jnp.zeros((DP - D, 128), f32)], axis=0).astype(bf16)
                r_ref[ib, :, j * 128:(j + 1) * 128] = _rb(jnp.dot(wrow, xnp, preferred_element_type=f32)[0:1, :])
                xn_ref[ib, j * 128:(j + 1) * 128, :] = xnp.T

        def layernorm_block(ib):
            layernorm_tiles(ib, range(NTQ))

        def qproj(ib, hh):
            xn = xn_ref[ib][:, :D]
            q = jnp.dot(xn, wq_ref[hh], preferred_element_type=f32) * QSCALE
            q = q.astype(bf16)
            for hh2 in range(2):
                for n in range(NTQ):
                    q_ref[hh2, n * 64:(n + 1) * 64, :] = _pk(q[n * 128:(n + 1) * 128, hh2 * DH:(hh2 + 1) * DH].T)

        def oproj(ib, hh, jobs=None):
            upd = jnp.dot(wo_ref[hh], jnp.concatenate([_upk(oc_ref[n]) for n in range(NTQ)], axis=1),
                          preferred_element_type=f32)
            if jobs is not None:
                jobs.append(upd[D - 1:D, :])
            for n in range(NTQ):
                acc_ref[ib * NTQ + n] = acc_ref[ib * NTQ + n] + upd[:, n * 128:(n + 1) * 128]

        def epilogue(ib):
            for j in range(NTQ):
                x = xs_ref[ib, :, j * 128:(j + 1) * 128].astype(f32)
                xs_ref[ib, :, j * 128:(j + 1) * 128] = (x + acc_ref[ib * NTQ + j] * g_ref[ib * NTQ + j]).astype(bf16)
            cp_out(ib).start()

        def topk():
            r = jnp.concatenate([r_ref[j] for j in range(NQ)], axis=0)
            ids = (lax.broadcasted_iota(jnp.int32, (NQ, MQ), 0) * MQ
                   + lax.broadcasted_iota(jnp.int32, (NQ, MQ), 1))
            rb = lax.shift_right_arithmetic(lax.bitcast_convert_type(r + 0.0, jnp.int32), 16)
            mono = jnp.where(rb < 0, -32769 - rb, rb) + 32768
            key = mono * S + (S - 1 - ids)
            keys = []
            for c in range(C):
                mx = jnp.max(jnp.max(key, axis=1, keepdims=True), axis=0, keepdims=True)
                key = jnp.where(key == mx, -1, key)
                keys.append(mx)
                idx_ref[c] = S - 1 - mx[0, 0] % S
            kv = jnp.concatenate(keys, axis=0)
            mono_s = kv // S - 32768
            rb_s = jnp.where(mono_s < 0, -32769 - mono_s, mono_s)
            rsel_ref[...] = jnp.broadcast_to(lax.bitcast_convert_type(lax.shift_left(rb_s, 16), f32), (C, 128))

        def moe():
            for cp in cp_moe():
                cp.wait()
            rows = []
            sel = []
            sub = lax.broadcasted_iota(jnp.int32, (16, DP), 0)
            for c in range(C):
                idx_s = jnp.clip(idx_ref[c], 0, S - 1)
                ib = idx_s // MQ
                off = idx_s - ib * MQ
                base = pl.multiple_of((off // 16) * 16, 16)
                blk = xn_ref[ib, pl.ds(base, 16), :].astype(f32)
                rows.append(jnp.sum(jnp.where(sub == off - base, blk, 0.0), axis=0, keepdims=True))
                sel.append(idx_s)
            rsel = rsel_ref[:, 0:1]
            xsel = jnp.concatenate(rows, axis=0)
            xs16 = jnp.concatenate([xsel, xsel], axis=0)[:, :D].astype(bf16)
            gt = _rb(jnp.dot(xs16, wg_ref[...], preferred_element_type=f32))
            u = _rb(jnp.dot(xs16, wu_ref[...], preferred_element_type=f32))
            hh = (_rb(_silu(gt)) * u).astype(bf16)
            y = _rb(lax.dot_general(hh, wdt_ref[...], NT, preferred_element_type=f32))[:C]
            y = _rb(y * _rb(_sigmoid(rsel)))
            gsel = _silu(_rb(xsel[:, :D] + y))
            gpad = jnp.concatenate([gsel, jnp.zeros((C, DP - D), f32)], axis=1)
            gpad = jnp.concatenate([gpad, jnp.zeros((128 - C, DP), f32)], axis=0)
            gt_all = gpad.T[:D]
            lane = lax.broadcasted_iota(jnp.int32, (D, 128), 1)
            for c in range(C):
                idx_s = sel[c]
                tt = idx_s // 128
                if mstore:
                    pltpu.store(g_ref.at[tt], jnp.broadcast_to(gt_all[:, c:c + 1], (D, 128)), mask=lane == idx_s - tt * 128)
                else:
                    g_ref[tt] = jnp.where(lane == idx_s - tt * 128, gt_all[:, c:c + 1], g_ref[tt])

        w1 = [cp_x(0), cp_v(0), cp_wq(0)]
        w2 = [cp_x(1), cp_k(0)] + ([] if late else [cp_v(1), cp_wo(0)])
        w3 = ([cp_v(1), cp_wo(0)] if late else []) + [cp_wq(1)] + [cp_x(ib) for ib in range(2, NQ)]
        if pro == 1:
            first, second, third = w1 + w2 + w3, [], []
        elif pro == 2:
            first, second, third = w1, w2, w3
        elif pro == 3:
            first, second, third = w1, w2 + w3, []
        elif pro == 4:
            first, second, third = w1 + w2, [], w3
        elif pro == 5:
            first, second, third = w1[:1], w1[1:] + w2, w3
        for cp in first:
            cp.start()
        z_ref[0] = 0
        r_ref[...] = jnp.zeros(r_ref.shape, f32)

        def zero_acc(j, c):
            acc_ref[j] = jnp.zeros((D, 128), f32)
            return c
        lax.fori_loop(0, NL, zero_acc, 0)
        wr = wr_ref[...].reshape(1, D)
        wr = jnp.concatenate([wr, jnp.zeros((1, DP - D), bf16)], axis=1)
        wrow_ref[...] = jnp.broadcast_to(wr.astype(f32), (16, DP)).astype(bf16)
        cp_x(0).wait()
        for cp in second:
            cp.start()
        layernorm_tiles(0, range(split))
        cp_v(0).wait()
        if waitall:
            cp_wq(0).wait()
        layernorm_tiles(0, range(split, NTQ))
        for j in range(NKT):
            vt_ref[0, j] = _pk(v_ref[0, j * 128:(j + 1) * 128, :].T)
        if not waitall:
            cp_wq(0).wait()
        if ln1 == 1:
            cp_x(1).wait()
            qproj(0, 0)
            layernorm_block(1)
        elif ln1 == 2:
            cp_x(1).wait()
            layernorm_block(1)
            qproj(0, 0)
        else:
            qproj(0, 0)
        for cp in third:
            cp.start()
        for h in range(1, H_EARLY):
            for cp in group(h):
                cp.start()

        def final_block():
            ib = NQ - 1
            upd = jnp.dot(wo_ref[HKV - 1], jnp.concatenate([_upk(oc_ref[n]) for n in range(NTQ)], axis=1),
                          preferred_element_type=f32)
            RR = D // rc
            for c in range(rc):
                rows = slice(c * RR, (c + 1) * RR)
                for n in range(NTQ):
                    cols = slice(n * 128, (n + 1) * 128)
                    sv = acc_ref[ib * NTQ + n, rows, :] + upd[rows, cols]
                    x = xs_ref[ib, rows, cols].astype(f32)
                    xs_ref[ib, rows, cols] = (x + sv * g_ref[ib * NTQ + n, rows, :]).astype(bf16)
                cp_tail(c).start()

        def main_block(t, carry, first=False, last=False):
            h = t // NQ
            i = t % NQ
            i_next = (t + 1) % NQ
            h_next = (t + 1) // NQ
            i_prev = (t - 1) % NQ
            h_prev = (t - 1) // NQ
            hv = jnp.minimum(h + 1, HKV - 1)
            z = z_ref[0]
            cur = h % 2
            st = {}
            jobs = []

            def qk(name, s_ref, col):
                q = jnp.concatenate([_upk(q_ref[col, n * 64:(n + 1) * 64, :]) for n in range(NTQ)], axis=1)
                m = None
                for j in range(S // KBQ):
                    ks = slice(j * KBQ, (j + 1) * KBQ)
                    s = jnp.dot(k_ref[h, ks, :], q, preferred_element_type=f32)
                    for n in range(NTQ):
                        s_ref[n, ks, :] = s[:, n * 128:(n + 1) * 128]
                    mj = jnp.max(s.reshape(KBQ // 8, 8, MQ), axis=0)
                    m = mj if m is None else jnp.maximum(m, mj)
                st[name] = jnp.max(m, axis=0, keepdims=True)
                jobs.append(st[name])

            def pv(name, s_ref, col):
                acc = None
                m = st[name]
                if name == "a":
                    m = m + jnp.minimum(jnp.abs(st["b"]), 0.0)
                l = None
                for j in range(S // KBP):
                    kd = pl.ds(pl.multiple_of(z + j * KBP, KBP), KBP)
                    sv = jnp.concatenate([s_ref[n, kd, :] for n in range(NTQ)], axis=1)
                    mg = m
                    if lag and len(jobs) >= lag:
                        mg = m + jnp.minimum(jnp.abs(jobs[-lag]), 0.0)
                    p = jnp.exp2(sv - mg)
                    lj = _tree(p, jnp.add)
                    l = lj if l is None else l + lj
                    pb = p.astype(bf16)
                    vt = jnp.concatenate([_upk(vt_ref[cur, jj]) for jj in range(j * KBP // 128, (j + 1) * KBP // 128)], axis=1)
                    oj = jnp.dot(vt, pb, preferred_element_type=f32)
                    jobs.append(oj[DH - 1:DH, :])
                    acc = oj if acc is None else acc + oj
                l = jnp.sum(l, axis=0, keepdims=True)
                ob = (acc * (1.0 / l)).astype(bf16)
                for n in range(NTQ):
                    oc_ref[n, col * DH // 2:(col + 1) * DH // 2, :] = _pk(ob[:, n * 128:(n + 1) * 128])

            def vtrans():
                for jj in range(VP // 128):
                    off = pl.multiple_of(i * VP + jj * 128, 128)
                    vt_ref[1 - cur, i * (VP // 128) + jj] = _pk(v_ref[hv, pl.ds(off, 128), :].T)

            for o in order.split(","):
                if o == "qa": qk("a", sa_ref, 0)
                elif o == "qb": qk("b", sb_ref, 1)
                elif o == "pa": pv("a", sa_ref, 0)
                elif o == "pb": pv("b", sb_ref, 1)
                elif o == "op":
                    if not first:
                        oproj(i_prev, h_prev, jobs)
                    if last:
                        epilogue(NQ - 2)
                elif o == "qp":
                    if not last:
                        qproj(i_next, h_next)
                elif o == "vt":
                    if not last:
                        vtrans()
            if last:
                final_block()
            return carry

        def single_block(t, carry):
            if topk_filler:
                topk()
            return main_block(t, carry)

        def multi_block(p, carry):
            for u in range(U):
                main_block(U * p + u, carry)
            return carry

        if not ln1:
            cp_x(1).wait()
            layernorm_block(1)
        cp_k(0).wait()
        cp_v(1).wait()
        main_block(0, 0, first=True)
        cp_wo(0).wait()

        TM = NQ + ((T - 2 - NQ) // U) * U
        starts = [1, 2, 3] + [h * NQ for h in range(1, H_EARLY)] + [MOE_T, TM, T - 2, T - 1]
        assert MOE_T == H_EARLY * NQ
        NSEG = len(starts) - 1
        SEG_MOE = NSEG - 3

        def segment(sg, carry):
            t0 = jnp.int32(0)
            t1 = jnp.int32(0)
            for k in range(NSEG):
                t0 = jnp.where(sg == k, starts[k], t0)
                t1 = jnp.where(sg == k, starts[k + 1], t1)
            paired = jnp.logical_and(sg >= NQ - 1, sg <= SEG_MOE)

            @pl.when(sg < NQ - 2)
            def _():
                cp_x(sg + 2).wait()
                layernorm_block(sg + 2)

            @pl.when(sg == NQ - 2)
            def _():
                cp_wq(1).wait()

            if bulk_seg >= 0:
                @pl.when(sg == bulk_seg)
                def _():
                    for h in range(H_EARLY, HKV):
                        for cp in group(h):
                            cp.start()

            if moe_dma_seg >= 0:
                @pl.when(sg == moe_dma_seg)
                def _():
                    for cp in cp_moe():
                        cp.start()

            for h in range(1, H_EARLY):
                @pl.when(sg == NQ - 2 + h)
                def _(h=h):
                    for cp in group(h):
                        cp.wait()

            @pl.when(sg == SEG_MOE)
            def _():
                for h in range(H_EARLY, HKV):
                    for cp in group(h):
                        cp.wait()
                if not topk_filler:
                    topk()
                moe()

            @pl.when(sg == NSEG - 1)
            def _():
                epilogue(0)

            p0 = jnp.where(paired, t0 // U, 0)
            p1 = jnp.where(paired, t1 // U, 0)
            lax.fori_loop(p0, p1, multi_block, 0)
            lax.fori_loop(jnp.where(paired, 0, t0), jnp.where(paired, 0, t1), single_block, 0)
            return carry

        lax.fori_loop(0, NSEG, segment, 0)
        epilogue(1)
        main_block(T - 1, 0, last=True)
        for ib in range(NQ - 1):
            cp_out(ib).wait()
        for c in range(rc):
            cp_tail(c).wait()

    def fn(A_x, A_k_cache, A_v_cache, A_wq, A_wo, B_x, B_w_r, B_w_gate, B_w_up, B_w_down):
        xt = A_x.reshape(S, D).T
        anyspec = pl.BlockSpec(memory_space=pl.ANY)
        out = pl.pallas_call(
            kernel,
            in_specs=[anyspec, anyspec, anyspec, anyspec, anyspec,
                      pl.BlockSpec(memory_space=pltpu.VMEM),
                      anyspec, anyspec, anyspec],
            out_specs=anyspec,
            out_shape=jax.ShapeDtypeStruct((D, S), bf16),
            scratch_shapes=[
                pltpu.VMEM((NQ, MQ, DP), bf16),
                pltpu.VMEM((NL, D, 128), f32),
                pltpu.VMEM((HKV, S, DH), bf16),
                pltpu.VMEM((HKV, S, DH), bf16),
                pltpu.VMEM((HKV, D, 2 * DH), bf16),
                pltpu.VMEM((HKV, D, 2 * DH), bf16),
                pltpu.VMEM((NTQ, S, 128), f32),
                pltpu.VMEM((NTQ, S, 128), f32),
                pltpu.VMEM((2, MQ // 2, DH), u32),
                pltpu.VMEM((NTQ, DH, 128), u32),
                pltpu.VMEM((2, NKT, DH // 2, 128), u32),
                pltpu.VMEM((NL, D, 128), f32),
                pltpu.VMEM((NQ, D, MQ), bf16),
                pltpu.VMEM((NQ, 1, MQ), f32),
                pltpu.VMEM((16, DP), bf16),
                pltpu.VMEM((D, F), bf16),
                pltpu.VMEM((D, F), bf16),
                pltpu.VMEM((D, F), bf16),
                pltpu.VMEM((C, 128), f32),
                pltpu.SMEM((1,), jnp.int32),
                pltpu.SMEM((C,), jnp.int32),
                pltpu.SemaphoreType.DMA((NQ,)),
                pltpu.SemaphoreType.DMA((HKV,)),
                pltpu.SemaphoreType.DMA((HKV,)),
                pltpu.SemaphoreType.DMA((HKV,)),
                pltpu.SemaphoreType.DMA((HKV,)),
                pltpu.SemaphoreType.DMA((3,)),
                pltpu.SemaphoreType.DMA((NQ,)),
                pltpu.SemaphoreType.DMA((4,)),
            ],
            compiler_params=pltpu.CompilerParams(
                vmem_limit_bytes=VL * 1024 * 1024),
            name="fused_attn_moe",
        )(xt, A_k_cache, A_v_cache, A_wq, A_wo.T, B_w_r, B_w_gate, B_w_up, B_w_down.T)
        return out.T.reshape(1, S, D)

    return fn


_fn = make_kernel()


@jax.jit
def pallas_recurrent_scan__gqa_block_cached__moe_arch_mod__prompt_kernel(
    A_x, A_k_cache, A_v_cache, A_wq, A_wo, B_x, B_w_r, B_w_gate, B_w_up, B_w_down):
    return _fn(A_x, A_k_cache, A_v_cache, A_wq, A_wo, B_x, B_w_r, B_w_gate, B_w_up, B_w_down)
```

```python
import functools
import jax
import jax.numpy as jnp
from jax import lax
import jax.experimental.pallas as pl
import jax.experimental.pallas.tpu as pltpu

S = 2048
D = 576
DP = 640
HQ = 32
HKV = 16
DH = 128
F = 4608
C = 8
LOG2E = 1.4426950408889634
QSCALE = (DH ** -0.5) * LOG2E
bf16 = jnp.bfloat16
f32 = jnp.float32
u32 = jnp.uint32
NT = (((1,), (1,)), ((), ()))


def _rb(x):
    return x.astype(bf16).astype(f32)


def _pk(x):
    return pltpu.bitcast(x, u32)


def _upk(x):
    return pltpu.bitcast(x, bf16)


def _sigmoid(x):
    return 0.5 * jnp.tanh(0.5 * x) + 0.5


def _silu(x):
    h = 0.5 * x
    return h * jnp.tanh(h) + h


def _lin(p, op, n=2):
    parts = [p[i * 8:(i + 1) * 8] for i in range(p.shape[0] // 8)]
    acc = parts[:n]
    for i in range(n, len(parts)):
        acc[i % n] = op(acc[i % n], parts[i])
    while len(acc) > 1:
        acc = [op(acc[i], acc[i + 1]) for i in range(0, len(acc), 2)]
    return acc[0]


def _tree(p, op):
    parts = [p[i * 8:(i + 1) * 8] for i in range(p.shape[0] // 8)]
    while len(parts) > 1:
        nxt = [op(parts[i], parts[i + 1]) for i in range(0, len(parts) - 1, 2)]
        if len(parts) % 2:
            nxt.append(parts[-1])
        parts = nxt
    return parts[0]


def make_kernel(MQ=512, KBQ=2048, KBP=128, VL=110, order="qa,qb,op,pa,qp,pb,vt", MOE_T=12, lag=5, pro=4, H_EARLY=3, moe_dma_seg=3, bulk_seg=0, waitall=True, topk_filler=True, split=2, mstore=True, U=2, late=False, ln1=0, rc=4, lastv=1):
    NQ = S // MQ
    NL = S // 128
    NTQ = MQ // 128
    T = HKV * NQ
    VP = S // NQ
    NKT = S // 128

    def kernel(xt_hbm, k_hbm, v_hbm, wq_hbm, wot_hbm, wr_ref, wg_hbm, wu_hbm, wdt_hbm,
               o_hbm,
               xn_ref, acc_ref, k_ref, v_ref, wq_ref, wo_ref,
               sa_ref, sb_ref, q_ref, oc_ref, vt_ref,
               g_ref, xs_ref, r_ref, wrow_ref, wg_ref, wu_ref, wdt_ref, rsel_ref, z_ref, idx_ref,
               sem_x, sem_k, sem_v, sem_wq, sem_wo, sem_m, sem_o, sem_t):

        def cp_x(ib):
            return pltpu.make_async_copy(xt_hbm.at[:, pl.ds(ib * MQ, MQ)], xs_ref.at[ib], sem_x.at[ib])

        def cp_k(h):
            return pltpu.make_async_copy(k_hbm.at[0, h], k_ref.at[h], sem_k.at[h])

        def cp_v(h):
            return pltpu.make_async_copy(v_hbm.at[0, h], v_ref.at[h], sem_v.at[h])

        def cp_wq(h):
            return pltpu.make_async_copy(wq_hbm.at[:, pl.ds(h * 256, 256)], wq_ref.at[h], sem_wq.at[h])

        def cp_wo(h):
            return pltpu.make_async_copy(wot_hbm.at[:, pl.ds(h * 256, 256)], wo_ref.at[h], sem_wo.at[h])

        def cp_moe():
            return [pltpu.make_async_copy(wg_hbm, wg_ref, sem_m.at[0]),
                    pltpu.make_async_copy(wu_hbm, wu_ref, sem_m.at[1]),
                    pltpu.make_async_copy(wdt_hbm, wdt_ref, sem_m.at[2])]

        def cp_out(ib):
            return pltpu.make_async_copy(xs_ref.at[ib], o_hbm.at[:, pl.ds(pl.multiple_of(ib * MQ, MQ), MQ)], sem_o.at[ib])

        def cp_tail(c):
            RR = D // rc
            return pltpu.make_async_copy(xs_ref.at[NQ - 1, pl.ds(c * RR, RR)],
                                         o_hbm.at[pl.ds(c * RR, RR), pl.ds((NQ - 1) * MQ, MQ)], sem_t.at[c])

        def group(h):
            cps = [cp_k(h), cp_wo(h)]
            if h + 1 < HKV:
                cps += [cp_v(h + 1), cp_wq(h + 1)]
            return cps

        def layernorm_tiles(ib, tiles):
            wrow = wrow_ref[...]
            for j in tiles:
                x = xs_ref[ib, :, j * 128:(j + 1) * 128].astype(f32)
                mean = jnp.sum(_lin(x, jnp.add), axis=0, keepdims=True) * (1.0 / D)
                xc = x - mean
                var = jnp.sum(_lin(xc * xc, jnp.add), axis=0, keepdims=True) * (1.0 / D)
                m = _rb(mean)
                inv = 1.0 / _rb(jnp.sqrt(_rb(_rb(var) + 1e-5)))
                xn = (x - m) * inv
                g_ref[ib * NTQ + j] = xn
                xnp = jnp.concatenate([xn, jnp.zeros((DP - D, 128), f32)], axis=0).astype(bf16)
                r_ref[ib, :, j * 128:(j + 1) * 128] = _rb(jnp.dot(wrow, xnp, preferred_element_type=f32)[0:1, :])
                xn_ref[ib, j * 128:(j + 1) * 128, :] = xnp.T

        def layernorm_block(ib):
            layernorm_tiles(ib, range(NTQ))

        def qproj(ib, hh):
            xn = xn_ref[ib][:, :D]
            q = jnp.dot(xn, wq_ref[hh], preferred_element_type=f32) * QSCALE
            q = q.astype(bf16)
            for hh2 in range(2):
                for n in range(NTQ):
                    q_ref[hh2, n * 64:(n + 1) * 64, :] = _pk(q[n * 128:(n + 1) * 128, hh2 * DH:(hh2 + 1) * DH].T)

        def oproj(ib, hh, jobs=None):
            upd = jnp.dot(wo_ref[hh], jnp.concatenate([_upk(oc_ref[n]) for n in range(NTQ)], axis=1),
                          preferred_element_type=f32)
            if jobs is not None:
                jobs.append(upd[D - 1:D, :])
            for n in range(NTQ):
                acc_ref[ib * NTQ + n] = acc_ref[ib * NTQ + n] + upd[:, n * 128:(n + 1) * 128]

        def epilogue(ib):
            for j in range(NTQ):
                x = xs_ref[ib, :, j * 128:(j + 1) * 128].astype(f32)
                xs_ref[ib, :, j * 128:(j + 1) * 128] = (x + acc_ref[ib * NTQ + j] * _silu(g_ref[ib * NTQ + j])).astype(bf16)
            cp_out(ib).start()

        def topk():
            r = jnp.concatenate([r_ref[j] for j in range(NQ)], axis=0)
            ids = (lax.broadcasted_iota(jnp.int32, (NQ, MQ), 0) * MQ
                   + lax.broadcasted_iota(jnp.int32, (NQ, MQ), 1))
            rb = lax.shift_right_arithmetic(lax.bitcast_convert_type(r + 0.0, jnp.int32), 16)
            mono = jnp.where(rb < 0, -32769 - rb, rb) + 32768
            key = mono * S + (S - 1 - ids)
            keys = []
            for c in range(C):
                mx = jnp.max(jnp.max(key, axis=1, keepdims=True), axis=0, keepdims=True)
                key = jnp.where(key == mx, -1, key)
                keys.append(mx)
                idx_ref[c] = S - 1 - mx[0, 0] % S
            kv = jnp.concatenate(keys, axis=0)
            mono_s = kv // S - 32768
            rb_s = jnp.where(mono_s < 0, -32769 - mono_s, mono_s)
            rsel_ref[...] = jnp.broadcast_to(lax.bitcast_convert_type(lax.shift_left(rb_s, 16), f32), (C, 128))

        def moe():
            for cp in cp_moe():
                cp.wait()
            rows = []
            sel = []
            sub = lax.broadcasted_iota(jnp.int32, (16, DP), 0)
            for c in range(C):
                idx_s = jnp.clip(idx_ref[c], 0, S - 1)
                ib = idx_s // MQ
                off = idx_s - ib * MQ
                base = pl.multiple_of((off // 16) * 16, 16)
                blk = xn_ref[ib, pl.ds(base, 16), :].astype(f32)
                rows.append(jnp.sum(jnp.where(sub == off - base, blk, 0.0), axis=0, keepdims=True))
                sel.append(idx_s)
            rsel = rsel_ref[:, 0:1]
            xsel = jnp.concatenate(rows, axis=0)
            xs16 = jnp.concatenate([xsel, xsel], axis=0)[:, :D].astype(bf16)
            gt = _rb(jnp.dot(xs16, wg_ref[...], preferred_element_type=f32))
            u = _rb(jnp.dot(xs16, wu_ref[...], preferred_element_type=f32))
            hh = (_rb(_silu(gt)) * u).astype(bf16)
            y = _rb(lax.dot_general(hh, wdt_ref[...], NT, preferred_element_type=f32))[:C]
            y = _rb(y * _rb(_sigmoid(rsel)))
            gsel = _rb(xsel[:, :D] + y)
            gpad = jnp.concatenate([gsel, jnp.zeros((C, DP - D), f32)], axis=1)
            gpad = jnp.concatenate([gpad, jnp.zeros((128 - C, DP), f32)], axis=0)
            gt_all = gpad.T[:D]
            lane = lax.broadcasted_iota(jnp.int32, (D, 128), 1)
            for c in range(C):
                idx_s = sel[c]
                tt = idx_s // 128
                if mstore:
                    pltpu.store(g_ref.at[tt], jnp.broadcast_to(gt_all[:, c:c + 1], (D, 128)), mask=lane == idx_s - tt * 128)
                else:
                    g_ref[tt] = jnp.where(lane == idx_s - tt * 128, gt_all[:, c:c + 1], g_ref[tt])

        w1 = [cp_x(0), cp_v(0), cp_wq(0)]
        w2 = [cp_x(1), cp_k(0)] + ([] if late else [cp_v(1), cp_wo(0)])
        w3 = ([cp_v(1), cp_wo(0)] if late else []) + [cp_wq(1)] + [cp_x(ib) for ib in range(2, NQ)]
        if pro == 1:
            first, second, third = w1 + w2 + w3, [], []
        elif pro == 2:
            first, second, third = w1, w2, w3
        elif pro == 3:
            first, second, third = w1, w2 + w3, []
        elif pro == 4:
            first, second, third = w1 + w2, [], w3
        elif pro == 5:
            first, second, third = w1[:1], w1[1:] + w2, w3
        for cp in first:
            cp.start()
        z_ref[0] = 0
        r_ref[...] = jnp.zeros(r_ref.shape, f32)

        def zero_acc(j, c):
            acc_ref[j] = jnp.zeros((D, 128), f32)
            return c
        lax.fori_loop(0, NL, zero_acc, 0)
        wr = wr_ref[...].reshape(1, D)
        wr = jnp.concatenate([wr, jnp.zeros((1, DP - D), bf16)], axis=1)
        wrow_ref[...] = jnp.broadcast_to(wr.astype(f32), (16, DP)).astype(bf16)
        cp_x(0).wait()
        for cp in second:
            cp.start()
        layernorm_tiles(0, range(split))
        cp_v(0).wait()
        if waitall:
            cp_wq(0).wait()
        layernorm_tiles(0, range(split, NTQ))
        for j in range(NKT):
            vt_ref[0, j] = _pk(v_ref[0, j * 128:(j + 1) * 128, :].T)
        if not waitall:
            cp_wq(0).wait()
        if ln1 == 1:
            cp_x(1).wait()
            qproj(0, 0)
            layernorm_block(1)
        elif ln1 == 2:
            cp_x(1).wait()
            layernorm_block(1)
            qproj(0, 0)
        else:
            qproj(0, 0)
        for cp in third:
            cp.start()
        for h in range(1, H_EARLY):
            for cp in group(h):
                cp.start()

        def final_block():
            ib = NQ - 1
            upd = jnp.dot(wo_ref[HKV - 1], jnp.concatenate([_upk(oc_ref[n]) for n in range(NTQ)], axis=1),
                          preferred_element_type=f32)
            RR = D // rc
            for c in range(rc):
                rows = slice(c * RR, (c + 1) * RR)
                for n in range(NTQ):
                    cols = slice(n * 128, (n + 1) * 128)
                    sv = acc_ref[ib * NTQ + n, rows, :] + upd[rows, cols]
                    x = xs_ref[ib, rows, cols].astype(f32)
                    xs_ref[ib, rows, cols] = (x + sv * _silu(g_ref[ib * NTQ + n, rows, :])).astype(bf16)
                cp_tail(c).start()

        def main_block(t, carry, first=False, last=False):
            h = t // NQ
            i = t % NQ
            i_next = (t + 1) % NQ
            h_next = (t + 1) // NQ
            i_prev = (t - 1) % NQ
            h_prev = (t - 1) // NQ
            hv = jnp.minimum(h + 1, HKV - 1)
            z = z_ref[0]
            cur = h % 2
            st = {}
            jobs = []

            def qk(name, s_ref, col):
                q = jnp.concatenate([_upk(q_ref[col, n * 64:(n + 1) * 64, :]) for n in range(NTQ)], axis=1)
                m = None
                for j in range(S // KBQ):
                    ks = slice(j * KBQ, (j + 1) * KBQ)
                    s = jnp.dot(k_ref[h, ks, :], q, preferred_element_type=f32)
                    for n in range(NTQ):
                        s_ref[n, ks, :] = s[:, n * 128:(n + 1) * 128]
                    mj = jnp.max(s.reshape(KBQ // 8, 8, MQ), axis=0)
                    m = mj if m is None else jnp.maximum(m, mj)
                st[name] = jnp.max(m, axis=0, keepdims=True)
                jobs.append(st[name])

            def pv(name, s_ref, col):
                acc = None
                m = st[name]
                if name == "a":
                    m = m + jnp.minimum(jnp.abs(st["b"]), 0.0)
                l = None
                for j in range(S // KBP):
                    kd = pl.ds(pl.multiple_of(z + j * KBP, KBP), KBP)
                    sv = jnp.concatenate([s_ref[n, kd, :] for n in range(NTQ)], axis=1)
                    mg = m
                    if lag and len(jobs) >= lag:
                        mg = m + jnp.minimum(jnp.abs(jobs[-lag]), 0.0)
                    p = jnp.exp2(sv - mg)
                    lj = _tree(p, jnp.add)
                    l = lj if l is None else l + lj
                    pb = p.astype(bf16)
                    vt = jnp.concatenate([_upk(vt_ref[cur, jj]) for jj in range(j * KBP // 128, (j + 1) * KBP // 128)], axis=1)
                    oj = jnp.dot(vt, pb, preferred_element_type=f32)
                    jobs.append(oj[DH - 1:DH, :])
                    acc = oj if acc is None else acc + oj
                l = jnp.sum(l, axis=0, keepdims=True)
                ob = (acc * (1.0 / l)).astype(bf16)
                for n in range(NTQ):
                    oc_ref[n, col * DH // 2:(col + 1) * DH // 2, :] = _pk(ob[:, n * 128:(n + 1) * 128])

            def vtrans():
                for jj in range(VP // 128):
                    off = pl.multiple_of(i * VP + jj * 128, 128)
                    vt_ref[1 - cur, i * (VP // 128) + jj] = _pk(v_ref[hv, pl.ds(off, 128), :].T)

            for o in order.split(","):
                if o == "qa": qk("a", sa_ref, 0)
                elif o == "qb": qk("b", sb_ref, 1)
                elif o == "pa":
                    pv("a", sa_ref, 0)
                    if last and lastv == 1:
                        epilogue(NQ - 2)
                    if last and lastv == 2:
                        epilogue(NQ - 3)
                        epilogue(NQ - 2)
                elif o == "pb": pv("b", sb_ref, 1)
                elif o == "op":
                    if not first:
                        oproj(i_prev, h_prev, jobs)
                    if last and lastv == 0:
                        epilogue(NQ - 2)
                elif o == "qp":
                    if not last:
                        qproj(i_next, h_next)
                elif o == "vt":
                    if not last:
                        vtrans()
            if last:
                final_block()
            return carry

        def single_block(t, carry):
            if topk_filler:
                topk()
            return main_block(t, carry)

        def multi_block(p, carry):
            for u in range(U):
                main_block(U * p + u, carry)
            return carry

        if not ln1:
            cp_x(1).wait()
            layernorm_block(1)
        cp_k(0).wait()
        cp_v(1).wait()
        main_block(0, 0, first=True)
        cp_wo(0).wait()

        TM = NQ + ((T - 2 - NQ) // U) * U
        starts = [1, 2, 3] + [h * NQ for h in range(1, H_EARLY)] + [MOE_T, TM, T - 2, T - 1]
        assert MOE_T == H_EARLY * NQ
        NSEG = len(starts) - 1
        SEG_MOE = NSEG - 3

        def segment(sg, carry):
            t0 = jnp.int32(0)
            t1 = jnp.int32(0)
            for k in range(NSEG):
                t0 = jnp.where(sg == k, starts[k], t0)
                t1 = jnp.where(sg == k, starts[k + 1], t1)
            paired = jnp.logical_and(sg >= NQ - 1, sg <= SEG_MOE)

            @pl.when(sg < NQ - 2)
            def _():
                cp_x(sg + 2).wait()
                layernorm_block(sg + 2)

            @pl.when(sg == NQ - 2)
            def _():
                cp_wq(1).wait()

            if bulk_seg >= 0:
                @pl.when(sg == bulk_seg)
                def _():
                    for h in range(H_EARLY, HKV):
                        for cp in group(h):
                            cp.start()

            if moe_dma_seg >= 0:
                @pl.when(sg == moe_dma_seg)
                def _():
                    for cp in cp_moe():
                        cp.start()

            for h in range(1, H_EARLY):
                @pl.when(sg == NQ - 2 + h)
                def _(h=h):
                    for cp in group(h):
                        cp.wait()

            @pl.when(sg == SEG_MOE)
            def _():
                for h in range(H_EARLY, HKV):
                    for cp in group(h):
                        cp.wait()
                if not topk_filler:
                    topk()
                moe()

            @pl.when(sg == NSEG - 1)
            def _():
                epilogue(0)

            p0 = jnp.where(paired, t0 // U, 0)
            p1 = jnp.where(paired, t1 // U, 0)
            lax.fori_loop(p0, p1, multi_block, 0)
            lax.fori_loop(jnp.where(paired, 0, t0), jnp.where(paired, 0, t1), single_block, 0)
            return carry

        lax.fori_loop(0, NSEG, segment, 0)
        if lastv == 1:
            @pl.when(z_ref[0] == 0)
            def _():
                epilogue(1)
        elif lastv == 0:
            epilogue(1)
        main_block(T - 1, 0, last=True)
        for ib in range(NQ - 1):
            cp_out(ib).wait()
        for c in range(rc):
            cp_tail(c).wait()

    def fn(A_x, A_k_cache, A_v_cache, A_wq, A_wo, B_x, B_w_r, B_w_gate, B_w_up, B_w_down):
        xt = A_x.reshape(S, D).T
        anyspec = pl.BlockSpec(memory_space=pl.ANY)
        out = pl.pallas_call(
            kernel,
            in_specs=[anyspec, anyspec, anyspec, anyspec, anyspec,
                      pl.BlockSpec(memory_space=pltpu.VMEM),
                      anyspec, anyspec, anyspec],
            out_specs=anyspec,
            out_shape=jax.ShapeDtypeStruct((D, S), bf16),
            scratch_shapes=[
                pltpu.VMEM((NQ, MQ, DP), bf16),
                pltpu.VMEM((NL, D, 128), f32),
                pltpu.VMEM((HKV, S, DH), bf16),
                pltpu.VMEM((HKV, S, DH), bf16),
                pltpu.VMEM((HKV, D, 2 * DH), bf16),
                pltpu.VMEM((HKV, D, 2 * DH), bf16),
                pltpu.VMEM((NTQ, S, 128), f32),
                pltpu.VMEM((NTQ, S, 128), f32),
                pltpu.VMEM((2, MQ // 2, DH), u32),
                pltpu.VMEM((NTQ, DH, 128), u32),
                pltpu.VMEM((2, NKT, DH // 2, 128), u32),
                pltpu.VMEM((NL, D, 128), f32),
                pltpu.VMEM((NQ, D, MQ), bf16),
                pltpu.VMEM((NQ, 1, MQ), f32),
                pltpu.VMEM((16, DP), bf16),
                pltpu.VMEM((D, F), bf16),
                pltpu.VMEM((D, F), bf16),
                pltpu.VMEM((D, F), bf16),
                pltpu.VMEM((C, 128), f32),
                pltpu.SMEM((1,), jnp.int32),
                pltpu.SMEM((C,), jnp.int32),
                pltpu.SemaphoreType.DMA((NQ,)),
                pltpu.SemaphoreType.DMA((HKV,)),
                pltpu.SemaphoreType.DMA((HKV,)),
                pltpu.SemaphoreType.DMA((HKV,)),
                pltpu.SemaphoreType.DMA((HKV,)),
                pltpu.SemaphoreType.DMA((3,)),
                pltpu.SemaphoreType.DMA((NQ,)),
                pltpu.SemaphoreType.DMA((4,)),
            ],
            compiler_params=pltpu.CompilerParams(
                vmem_limit_bytes=VL * 1024 * 1024),
            name="fused_attn_moe",
        )(xt, A_k_cache, A_v_cache, A_wq, A_wo.T, B_w_r, B_w_gate, B_w_up, B_w_down.T)
        return out.T.reshape(1, S, D)

    return fn


_fn = make_kernel()


@jax.jit
def pallas_recurrent_scan__gqa_block_cached__moe_arch_mod__prompt_kernel(
    A_x, A_k_cache, A_v_cache, A_wq, A_wo, B_x, B_w_r, B_w_gate, B_w_up, B_w_down):
    return _fn(A_x, A_k_cache, A_v_cache, A_wq, A_wo, B_x, B_w_r, B_w_gate, B_w_up, B_w_down)
```

```python
import functools
import jax
import jax.numpy as jnp
from jax import lax
import jax.experimental.pallas as pl
import jax.experimental.pallas.tpu as pltpu

S = 2048
D = 576
DP = 640
HQ = 32
HKV = 16
DH = 128
F = 4608
C = 8
LOG2E = 1.4426950408889634
QSCALE = (DH ** -0.5) * LOG2E
bf16 = jnp.bfloat16
f32 = jnp.float32
u32 = jnp.uint32
NT = (((1,), (1,)), ((), ()))


def _rb(x):
    return x.astype(bf16).astype(f32)


def _pk(x):
    return pltpu.bitcast(x, u32)


def _upk(x):
    return pltpu.bitcast(x, bf16)


def _sigmoid(x):
    return 0.5 * jnp.tanh(0.5 * x) + 0.5


def _silu(x):
    h = 0.5 * x
    return h * jnp.tanh(h) + h


def _lin(p, op, n=2):
    parts = [p[i * 8:(i + 1) * 8] for i in range(p.shape[0] // 8)]
    acc = parts[:n]
    for i in range(n, len(parts)):
        acc[i % n] = op(acc[i % n], parts[i])
    while len(acc) > 1:
        acc = [op(acc[i], acc[i + 1]) for i in range(0, len(acc), 2)]
    return acc[0]


def _tree(p, op):
    parts = [p[i * 8:(i + 1) * 8] for i in range(p.shape[0] // 8)]
    while len(parts) > 1:
        nxt = [op(parts[i], parts[i + 1]) for i in range(0, len(parts) - 1, 2)]
        if len(parts) % 2:
            nxt.append(parts[-1])
        parts = nxt
    return parts[0]


def make_kernel(MQ=512, KBQ=2048, KBP=128, VL=110, order="qa,qb,op,pa,qp,pb,vt", MOE_T=8, lag=5, pro=4, H_EARLY=2, moe_dma_seg=1, bulk_seg=0, waitall=True, topk_filler=True, split=2, mstore=True, U=2, late=False, ln1=0, rc=4, lastv=1):
    NQ = S // MQ
    NL = S // 128
    NTQ = MQ // 128
    T = HKV * NQ
    VP = S // NQ
    NKT = S // 128

    def kernel(xt_hbm, k_hbm, v_hbm, wq_hbm, wot_hbm, wr_ref, wg_hbm, wu_hbm, wdt_hbm,
               o_hbm,
               xn_ref, acc_ref, k_ref, v_ref, wq_ref, wo_ref,
               sa_ref, sb_ref, q_ref, oc_ref, vt_ref,
               g_ref, xs_ref, r_ref, wrow_ref, wg_ref, wu_ref, wdt_ref, rsel_ref, z_ref, idx_ref,
               sem_x, sem_k, sem_v, sem_wq, sem_wo, sem_m, sem_o, sem_t):

        def cp_x(ib):
            return pltpu.make_async_copy(xt_hbm.at[:, pl.ds(ib * MQ, MQ)], xs_ref.at[ib], sem_x.at[ib])

        def cp_k(h):
            return pltpu.make_async_copy(k_hbm.at[0, h], k_ref.at[h], sem_k.at[h])

        def cp_v(h):
            return pltpu.make_async_copy(v_hbm.at[0, h], v_ref.at[h], sem_v.at[h])

        def cp_wq(h):
            return pltpu.make_async_copy(wq_hbm.at[:, pl.ds(h * 256, 256)], wq_ref.at[h], sem_wq.at[h])

        def cp_wo(h):
            return pltpu.make_async_copy(wot_hbm.at[:, pl.ds(h * 256, 256)], wo_ref.at[h], sem_wo.at[h])

        def cp_moe():
            return [pltpu.make_async_copy(wg_hbm, wg_ref, sem_m.at[0]),
                    pltpu.make_async_copy(wu_hbm, wu_ref, sem_m.at[1]),
                    pltpu.make_async_copy(wdt_hbm, wdt_ref, sem_m.at[2])]

        def cp_out(ib):
            return pltpu.make_async_copy(xs_ref.at[ib], o_hbm.at[:, pl.ds(pl.multiple_of(ib * MQ, MQ), MQ)], sem_o.at[ib])

        def cp_tail(c):
            RR = D // rc
            return pltpu.make_async_copy(xs_ref.at[NQ - 1, pl.ds(c * RR, RR)],
                                         o_hbm.at[pl.ds(c * RR, RR), pl.ds((NQ - 1) * MQ, MQ)], sem_t.at[c])

        def group(h):
            cps = [cp_k(h), cp_wo(h)]
            if h + 1 < HKV:
                cps += [cp_v(h + 1), cp_wq(h + 1)]
            return cps

        def layernorm_tiles(ib, tiles):
            wrow = wrow_ref[...]
            for j in tiles:
                x = xs_ref[ib, :, j * 128:(j + 1) * 128].astype(f32)
                mean = jnp.sum(_lin(x, jnp.add), axis=0, keepdims=True) * (1.0 / D)
                xc = x - mean
                var = jnp.sum(_lin(xc * xc, jnp.add), axis=0, keepdims=True) * (1.0 / D)
                m = _rb(mean)
                inv = 1.0 / _rb(jnp.sqrt(_rb(_rb(var) + 1e-5)))
                xn = (x - m) * inv
                g_ref[ib * NTQ + j] = xn
                xnp = jnp.concatenate([xn, jnp.zeros((DP - D, 128), f32)], axis=0).astype(bf16)
                r_ref[ib, :, j * 128:(j + 1) * 128] = _rb(jnp.dot(wrow, xnp, preferred_element_type=f32)[0:1, :])
                xn_ref[ib, j * 128:(j + 1) * 128, :] = xnp.T

        def layernorm_block(ib):
            layernorm_tiles(ib, range(NTQ))

        def qproj(ib, hh):
            xn = xn_ref[ib][:, :D]
            q = jnp.dot(xn, wq_ref[hh], preferred_element_type=f32) * QSCALE
            q = q.astype(bf16)
            for hh2 in range(2):
                for n in range(NTQ):
                    q_ref[hh2, n * 64:(n + 1) * 64, :] = _pk(q[n * 128:(n + 1) * 128, hh2 * DH:(hh2 + 1) * DH].T)

        def oproj(ib, hh, jobs=None):
            upd = jnp.dot(wo_ref[hh], jnp.concatenate([_upk(oc_ref[n]) for n in range(NTQ)], axis=1),
                          preferred_element_type=f32)
            if jobs is not None:
                jobs.append(upd[D - 1:D, :])
            for n in range(NTQ):
                acc_ref[ib * NTQ + n] = acc_ref[ib * NTQ + n] + upd[:, n * 128:(n + 1) * 128]

        def epilogue(ib):
            sv = jnp.concatenate([acc_ref[ib * NTQ + j] for j in range(NTQ)], axis=1)
            bv = jnp.concatenate([g_ref[ib * NTQ + j] for j in range(NTQ)], axis=1)
            xs_ref[ib] = (xs_ref[ib].astype(f32) + sv * _silu(bv)).astype(bf16)
            cp_out(ib).start()

        def topk():
            r = jnp.concatenate([r_ref[j] for j in range(NQ)], axis=0)
            ids = (lax.broadcasted_iota(jnp.int32, (NQ, MQ), 0) * MQ
                   + lax.broadcasted_iota(jnp.int32, (NQ, MQ), 1))
            rb = lax.shift_right_arithmetic(lax.bitcast_convert_type(r + 0.0, jnp.int32), 16)
            mono = jnp.where(rb < 0, -32769 - rb, rb) + 32768
            key = mono * S + (S - 1 - ids)
            keys = []
            for c in range(C):
                mx = jnp.max(jnp.max(key, axis=1, keepdims=True), axis=0, keepdims=True)
                key = jnp.where(key == mx, -1, key)
                keys.append(mx)
                idx_ref[c] = S - 1 - mx[0, 0] % S
            kv = jnp.concatenate(keys, axis=0)
            mono_s = kv // S - 32768
            rb_s = jnp.where(mono_s < 0, -32769 - mono_s, mono_s)
            rsel_ref[...] = jnp.broadcast_to(lax.bitcast_convert_type(lax.shift_left(rb_s, 16), f32), (C, 128))

        def moe():
            for cp in cp_moe():
                cp.wait()
            rows = []
            sel = []
            sub = lax.broadcasted_iota(jnp.int32, (16, DP), 0)
            for c in range(C):
                idx_s = jnp.clip(idx_ref[c], 0, S - 1)
                ib = idx_s // MQ
                off = idx_s - ib * MQ
                base = pl.multiple_of((off // 16) * 16, 16)
                blk = xn_ref[ib, pl.ds(base, 16), :].astype(f32)
                rows.append(jnp.sum(jnp.where(sub == off - base, blk, 0.0), axis=0, keepdims=True))
                sel.append(idx_s)
            rsel = rsel_ref[:, 0:1]
            xsel = jnp.concatenate(rows, axis=0)
            xs16 = jnp.concatenate([xsel, xsel], axis=0)[:, :D].astype(bf16)
            gt = _rb(jnp.dot(xs16, wg_ref[...], preferred_element_type=f32))
            u = _rb(jnp.dot(xs16, wu_ref[...], preferred_element_type=f32))
            hh = (_rb(_silu(gt)) * u).astype(bf16)
            y = _rb(lax.dot_general(hh, wdt_ref[...], NT, preferred_element_type=f32))[:C]
            y = _rb(y * _rb(_sigmoid(rsel)))
            gsel = _rb(xsel[:, :D] + y)
            gpad = jnp.concatenate([gsel, jnp.zeros((C, DP - D), f32)], axis=1)
            gpad = jnp.concatenate([gpad, jnp.zeros((128 - C, DP), f32)], axis=0)
            gt_all = gpad.T[:D]
            lane = lax.broadcasted_iota(jnp.int32, (D, 128), 1)
            for c in range(C):
                idx_s = sel[c]
                tt = idx_s // 128
                if mstore:
                    pltpu.store(g_ref.at[tt], jnp.broadcast_to(gt_all[:, c:c + 1], (D, 128)), mask=lane == idx_s - tt * 128)
                else:
                    g_ref[tt] = jnp.where(lane == idx_s - tt * 128, gt_all[:, c:c + 1], g_ref[tt])

        w1 = [cp_x(0), cp_v(0), cp_wq(0)]
        w2 = [cp_x(1), cp_k(0)] + ([] if late else [cp_v(1), cp_wo(0)])
        w3 = ([cp_v(1), cp_wo(0)] if late else []) + [cp_wq(1)] + [cp_x(ib) for ib in range(2, NQ)]
        if pro == 1:
            first, second, third = w1 + w2 + w3, [], []
        elif pro == 2:
            first, second, third = w1, w2, w3
        elif pro == 3:
            first, second, third = w1, w2 + w3, []
        elif pro == 4:
            first, second, third = w1 + w2, [], w3
        elif pro == 5:
            first, second, third = w1[:1], w1[1:] + w2, w3
        for cp in first:
            cp.start()
        z_ref[0] = 0
        r_ref[...] = jnp.zeros(r_ref.shape, f32)

        def zero_acc(j, c):
            acc_ref[j] = jnp.zeros((D, 128), f32)
            return c
        lax.fori_loop(0, NL, zero_acc, 0)
        wr = wr_ref[...].reshape(1, D)
        wr = jnp.concatenate([wr, jnp.zeros((1, DP - D), bf16)], axis=1)
        wrow_ref[...] = jnp.broadcast_to(wr.astype(f32), (16, DP)).astype(bf16)
        cp_x(0).wait()
        for cp in second:
            cp.start()
        layernorm_tiles(0, range(split))
        cp_v(0).wait()
        if waitall:
            cp_wq(0).wait()
        layernorm_tiles(0, range(split, NTQ))
        for j in range(NKT):
            vt_ref[0, j] = _pk(v_ref[0, j * 128:(j + 1) * 128, :].T)
        if not waitall:
            cp_wq(0).wait()
        if ln1 == 1:
            cp_x(1).wait()
            qproj(0, 0)
            layernorm_block(1)
        elif ln1 == 2:
            cp_x(1).wait()
            layernorm_block(1)
            qproj(0, 0)
        else:
            qproj(0, 0)
        for cp in third:
            cp.start()
        for h in range(1, H_EARLY):
            for cp in group(h):
                cp.start()

        def final_block():
            ib = NQ - 1
            upd = jnp.dot(wo_ref[HKV - 1], jnp.concatenate([_upk(oc_ref[n]) for n in range(NTQ)], axis=1),
                          preferred_element_type=f32)
            RR = D // rc
            for c in range(rc):
                rows = slice(c * RR, (c + 1) * RR)
                sv = jnp.concatenate([acc_ref[ib * NTQ + n, rows, :] for n in range(NTQ)], axis=1) + upd[rows, :]
                bv = jnp.concatenate([g_ref[ib * NTQ + n, rows, :] for n in range(NTQ)], axis=1)
                xs_ref[ib, rows, :] = (xs_ref[ib, rows, :].astype(f32) + sv * _silu(bv)).astype(bf16)
                cp_tail(c).start()

        def main_block(t, carry, first=False, last=False):
            h = t // NQ
            i = t % NQ
            i_next = (t + 1) % NQ
            h_next = (t + 1) // NQ
            i_prev = (t - 1) % NQ
            h_prev = (t - 1) // NQ
            hv = jnp.minimum(h + 1, HKV - 1)
            z = z_ref[0]
            cur = h % 2
            st = {}
            jobs = []

            def qk(name, s_ref, col):
                q = jnp.concatenate([_upk(q_ref[col, n * 64:(n + 1) * 64, :]) for n in range(NTQ)], axis=1)
                m = None
                for j in range(S // KBQ):
                    ks = slice(j * KBQ, (j + 1) * KBQ)
                    s = jnp.dot(k_ref[h, ks, :], q, preferred_element_type=f32)
                    for n in range(NTQ):
                        s_ref[n, ks, :] = s[:, n * 128:(n + 1) * 128]
                    mj = jnp.max(s.reshape(KBQ // 8, 8, MQ), axis=0)
                    m = mj if m is None else jnp.maximum(m, mj)
                st[name] = jnp.max(m, axis=0, keepdims=True)
                jobs.append(st[name])

            def pv(name, s_ref, col):
                acc = None
                m = st[name]
                if name == "a":
                    m = m + jnp.minimum(jnp.abs(st["b"]), 0.0)
                l = None
                for j in range(S // KBP):
                    kd = pl.ds(pl.multiple_of(z + j * KBP, KBP), KBP)
                    sv = jnp.concatenate([s_ref[n, kd, :] for n in range(NTQ)], axis=1)
                    mg = m
                    if lag and len(jobs) >= lag:
                        mg = m + jnp.minimum(jnp.abs(jobs[-lag]), 0.0)
                    p = jnp.exp2(sv - mg)
                    lj = _tree(p, jnp.add)
                    l = lj if l is None else l + lj
                    pb = p.astype(bf16)
                    vt = jnp.concatenate([_upk(vt_ref[cur, jj]) for jj in range(j * KBP // 128, (j + 1) * KBP // 128)], axis=1)
                    oj = jnp.dot(vt, pb, preferred_element_type=f32)
                    jobs.append(oj[DH - 1:DH, :])
                    acc = oj if acc is None else acc + oj
                l = jnp.sum(l, axis=0, keepdims=True)
                ob = (acc * (1.0 / l)).astype(bf16)
                for n in range(NTQ):
                    oc_ref[n, col * DH // 2:(col + 1) * DH // 2, :] = _pk(ob[:, n * 128:(n + 1) * 128])

            def vtrans():
                for jj in range(VP // 128):
                    off = pl.multiple_of(i * VP + jj * 128, 128)
                    vt_ref[1 - cur, i * (VP // 128) + jj] = _pk(v_ref[hv, pl.ds(off, 128), :].T)

            for o in order.split(","):
                if o == "qa": qk("a", sa_ref, 0)
                elif o == "qb": qk("b", sb_ref, 1)
                elif o == "pa":
                    pv("a", sa_ref, 0)
                    if last and lastv == 1:
                        epilogue(NQ - 2)
                    if last and lastv == 2:
                        epilogue(NQ - 3)
                        epilogue(NQ - 2)
                elif o == "pb": pv("b", sb_ref, 1)
                elif o == "op":
                    if not first:
                        oproj(i_prev, h_prev, jobs)
                    if last and lastv == 0:
                        epilogue(NQ - 2)
                elif o == "qp":
                    if not last:
                        qproj(i_next, h_next)
                elif o == "vt":
                    if not last:
                        vtrans()
            if last:
                final_block()
            return carry

        def single_block(t, carry):
            if topk_filler:
                topk()
            return main_block(t, carry)

        def multi_block(p, carry):
            for u in range(U):
                main_block(U * p + u, carry)
            return carry

        if not ln1:
            cp_x(1).wait()
            layernorm_block(1)
        cp_k(0).wait()
        cp_v(1).wait()
        main_block(0, 0, first=True)
        cp_wo(0).wait()

        TM = NQ + ((T - 2 - NQ) // U) * U
        assert TM == T - 2
        starts = [1, 2] + [h * NQ for h in range(1, H_EARLY)] + [MOE_T, T - 2, T - 1]
        assert MOE_T == H_EARLY * NQ and U == 2
        NSEG = len(starts) - 1
        SEG_MOE = NSEG - 2

        def segment(sg, carry):
            t0 = jnp.int32(0)
            t1 = jnp.int32(0)
            for k in range(NSEG):
                t0 = jnp.where(sg == k, starts[k], t0)
                t1 = jnp.where(sg == k, starts[k + 1], t1)
            paired = jnp.logical_and(sg >= 1, sg <= SEG_MOE)

            @pl.when(sg == 0)
            def _():
                for h in range(H_EARLY, HKV):
                    for cp in group(h):
                        cp.start()

                def ln(ib, c):
                    cp_x(ib).wait()
                    layernorm_block(ib)
                    return c
                lax.fori_loop(2, NQ, ln, 0)

            @pl.when(sg == 1)
            def _():
                cp_wq(1).wait()

            @pl.when(sg == moe_dma_seg)
            def _():
                for cp in cp_moe():
                    cp.start()

            for h in range(1, H_EARLY):
                @pl.when(sg == 1 + h)
                def _(h=h):
                    for cp in group(h):
                        cp.wait()

            @pl.when(sg == SEG_MOE)
            def _():
                for h in range(H_EARLY, HKV):
                    for cp in group(h):
                        cp.wait()
                if not topk_filler:
                    topk()
                moe()

            @pl.when(sg == NSEG - 1)
            def _():
                epilogue(0)

            p0 = jnp.where(paired, t0 // U, 0)
            p1 = jnp.where(paired, t1 // U, 0)
            lax.fori_loop(p0, p1, multi_block, 0)
            lax.fori_loop(jnp.where(paired, 0, t0), jnp.where(paired, 0, t1), single_block, 0)
            return carry

        lax.fori_loop(0, NSEG, segment, 0)
        if lastv == 1:
            @pl.when(z_ref[0] == 0)
            def _():
                epilogue(1)
        elif lastv == 0:
            epilogue(1)
        main_block(T - 1, 0, last=True)
        for ib in range(NQ - 1):
            cp_out(ib).wait()
        for c in range(rc):
            cp_tail(c).wait()

    def fn(A_x, A_k_cache, A_v_cache, A_wq, A_wo, B_x, B_w_r, B_w_gate, B_w_up, B_w_down):
        xt = A_x.reshape(S, D).T
        anyspec = pl.BlockSpec(memory_space=pl.ANY)
        out = pl.pallas_call(
            kernel,
            in_specs=[anyspec, anyspec, anyspec, anyspec, anyspec,
                      pl.BlockSpec(memory_space=pltpu.VMEM),
                      anyspec, anyspec, anyspec],
            out_specs=anyspec,
            out_shape=jax.ShapeDtypeStruct((D, S), bf16),
            scratch_shapes=[
                pltpu.VMEM((NQ, MQ, DP), bf16),
                pltpu.VMEM((NL, D, 128), f32),
                pltpu.VMEM((HKV, S, DH), bf16),
                pltpu.VMEM((HKV, S, DH), bf16),
                pltpu.VMEM((HKV, D, 2 * DH), bf16),
                pltpu.VMEM((HKV, D, 2 * DH), bf16),
                pltpu.VMEM((NTQ, S, 128), f32),
                pltpu.VMEM((NTQ, S, 128), f32),
                pltpu.VMEM((2, MQ // 2, DH), u32),
                pltpu.VMEM((NTQ, DH, 128), u32),
                pltpu.VMEM((2, NKT, DH // 2, 128), u32),
                pltpu.VMEM((NL, D, 128), f32),
                pltpu.VMEM((NQ, D, MQ), bf16),
                pltpu.VMEM((NQ, 1, MQ), f32),
                pltpu.VMEM((16, DP), bf16),
                pltpu.VMEM((D, F), bf16),
                pltpu.VMEM((D, F), bf16),
                pltpu.VMEM((D, F), bf16),
                pltpu.VMEM((C, 128), f32),
                pltpu.SMEM((1,), jnp.int32),
                pltpu.SMEM((C,), jnp.int32),
                pltpu.SemaphoreType.DMA((NQ,)),
                pltpu.SemaphoreType.DMA((HKV,)),
                pltpu.SemaphoreType.DMA((HKV,)),
                pltpu.SemaphoreType.DMA((HKV,)),
                pltpu.SemaphoreType.DMA((HKV,)),
                pltpu.SemaphoreType.DMA((3,)),
                pltpu.SemaphoreType.DMA((NQ,)),
                pltpu.SemaphoreType.DMA((4,)),
            ],
            compiler_params=pltpu.CompilerParams(
                vmem_limit_bytes=VL * 1024 * 1024),
            name="fused_attn_moe",
        )(xt, A_k_cache, A_v_cache, A_wq, A_wo.T, B_w_r, B_w_gate, B_w_up, B_w_down.T)
        return out.T.reshape(1, S, D)

    return fn


_fn = make_kernel()


@jax.jit
def pallas_recurrent_scan__gqa_block_cached__moe_arch_mod__prompt_kernel(
    A_x, A_k_cache, A_v_cache, A_wq, A_wo, B_x, B_w_r, B_w_gate, B_w_up, B_w_down):
    return _fn(A_x, A_k_cache, A_v_cache, A_wq, A_wo, B_x, B_w_r, B_w_gate, B_w_up, B_w_down)
```

```python
import jax
import jax.numpy as jnp
from jax import lax
import jax.experimental.pallas as pl
import jax.experimental.pallas.tpu as pltpu

S = 2048
D = 576
DP = 640
HKV = 16
DH = 128
F = 4608
C = 8
MQ = 512
KBP = 128
LAG = 5
MOE_T = 12
RC = 4
VMEM_LIMIT = 110 * 1024 * 1024

NQ = S // MQ
NL = S // 128
NTQ = MQ // 128
NKT = S // 128
VP = S // NQ
T = HKV * NQ
H_EARLY = MOE_T // NQ
QSCALE = (DH ** -0.5) * 1.4426950408889634

bf16 = jnp.bfloat16
f32 = jnp.float32
u32 = jnp.uint32
NT = (((1,), (1,)), ((), ()))


def _rb(x):
    return x.astype(bf16).astype(f32)


def _pk(x):
    return pltpu.bitcast(x, u32)


def _upk(x):
    return pltpu.bitcast(x, bf16)


def _sigmoid(x):
    return 0.5 * jnp.tanh(0.5 * x) + 0.5


def _silu(x):
    h = 0.5 * x
    return h * jnp.tanh(h) + h


def _lin(p, op, n=2):
    parts = [p[i * 8:(i + 1) * 8] for i in range(p.shape[0] // 8)]
    acc = parts[:n]
    for i in range(n, len(parts)):
        acc[i % n] = op(acc[i % n], parts[i])
    while len(acc) > 1:
        acc = [op(acc[i], acc[i + 1]) for i in range(0, len(acc), 2)]
    return acc[0]


def _tree(p, op):
    parts = [p[i * 8:(i + 1) * 8] for i in range(p.shape[0] // 8)]
    while len(parts) > 1:
        nxt = [op(parts[i], parts[i + 1]) for i in range(0, len(parts) - 1, 2)]
        if len(parts) % 2:
            nxt.append(parts[-1])
        parts = nxt
    return parts[0]


def _zero_after(x):
    return jnp.minimum(jnp.abs(x), 0.0)


def _kernel(xt_hbm, k_hbm, v_hbm, wq_hbm, wot_hbm, wr_ref, wg_hbm, wu_hbm, wdt_hbm,
            o_hbm,
            xn_ref, acc_ref, k_ref, v_ref, wq_ref, wo_ref,
            sa_ref, sb_ref, q_ref, oc_ref, vt_ref,
            g_ref, xs_ref, r_ref, wrow_ref, wg_ref, wu_ref, wdt_ref, rsel_ref, z_ref, idx_ref,
            sem_x, sem_k, sem_v, sem_wq, sem_wo, sem_m, sem_o, sem_t):

    def cp_x(ib):
        return pltpu.make_async_copy(xt_hbm.at[:, pl.ds(ib * MQ, MQ)], xs_ref.at[ib], sem_x.at[ib])

    def cp_k(h):
        return pltpu.make_async_copy(k_hbm.at[0, h], k_ref.at[h], sem_k.at[h])

    def cp_v(h):
        return pltpu.make_async_copy(v_hbm.at[0, h], v_ref.at[h], sem_v.at[h])

    def cp_wq(h):
        return pltpu.make_async_copy(wq_hbm.at[:, pl.ds(h * 256, 256)], wq_ref.at[h], sem_wq.at[h])

    def cp_wo(h):
        return pltpu.make_async_copy(wot_hbm.at[:, pl.ds(h * 256, 256)], wo_ref.at[h], sem_wo.at[h])

    def cp_moe():
        return [pltpu.make_async_copy(wg_hbm, wg_ref, sem_m.at[0]),
                pltpu.make_async_copy(wu_hbm, wu_ref, sem_m.at[1]),
                pltpu.make_async_copy(wdt_hbm, wdt_ref, sem_m.at[2])]

    def cp_out(ib):
        return pltpu.make_async_copy(xs_ref.at[ib], o_hbm.at[:, pl.ds(pl.multiple_of(ib * MQ, MQ), MQ)], sem_o.at[ib])

    def cp_tail(c):
        rr = D // RC
        return pltpu.make_async_copy(xs_ref.at[NQ - 1, pl.ds(c * rr, rr)],
                                     o_hbm.at[pl.ds(c * rr, rr), pl.ds((NQ - 1) * MQ, MQ)], sem_t.at[c])

    def group(h):
        cps = [cp_k(h), cp_wo(h)]
        if h + 1 < HKV:
            cps += [cp_v(h + 1), cp_wq(h + 1)]
        return cps

    def layernorm_tiles(ib, tiles):
        wrow = wrow_ref[...]
        for j in tiles:
            x = xs_ref[ib, :, j * 128:(j + 1) * 128].astype(f32)
            mean = jnp.sum(_lin(x, jnp.add), axis=0, keepdims=True) * (1.0 / D)
            xc = x - mean
            var = jnp.sum(_lin(xc * xc, jnp.add), axis=0, keepdims=True) * (1.0 / D)
            m = _rb(mean)
            inv = 1.0 / _rb(jnp.sqrt(_rb(_rb(var) + 1e-5)))
            xn = _rb(x - m) * inv
            g_ref[ib * NTQ + j] = xn
            xnp = jnp.concatenate([xn, jnp.zeros((DP - D, 128), f32)], axis=0).astype(bf16)
            r_ref[ib, :, j * 128:(j + 1) * 128] = _rb(jnp.dot(wrow, xnp, preferred_element_type=f32)[0:1, :])
            xn_ref[ib, j * 128:(j + 1) * 128, :] = xnp.T

    def layernorm_block(ib):
        layernorm_tiles(ib, range(NTQ))

    def qproj(ib, hh):
        xn = xn_ref[ib][:, :D]
        q = jnp.dot(xn, wq_ref[hh], preferred_element_type=f32) * QSCALE
        q = q.astype(bf16)
        for hh2 in range(2):
            for n in range(NTQ):
                q_ref[hh2, n * 64:(n + 1) * 64, :] = _pk(q[n * 128:(n + 1) * 128, hh2 * DH:(hh2 + 1) * DH].T)

    def oproj(ib, hh, jobs):
        upd = jnp.dot(wo_ref[hh], jnp.concatenate([_upk(oc_ref[n]) for n in range(NTQ)], axis=1),
                      preferred_element_type=f32)
        jobs.append(upd[D - 1:D, :])
        for n in range(NTQ):
            acc_ref[ib * NTQ + n] = acc_ref[ib * NTQ + n] + upd[:, n * 128:(n + 1) * 128]

    def epilogue(ib):
        sv = jnp.concatenate([acc_ref[ib * NTQ + j] for j in range(NTQ)], axis=1)
        bv = jnp.concatenate([g_ref[ib * NTQ + j] for j in range(NTQ)], axis=1)
        xs_ref[ib] = (xs_ref[ib].astype(f32) + sv * _silu(bv)).astype(bf16)
        cp_out(ib).start()

    def final_block():
        ib = NQ - 1
        upd = jnp.dot(wo_ref[HKV - 1], jnp.concatenate([_upk(oc_ref[n]) for n in range(NTQ)], axis=1),
                      preferred_element_type=f32)
        rr = D // RC
        for c in range(RC):
            rows = slice(c * rr, (c + 1) * rr)
            sv = jnp.concatenate([acc_ref[ib * NTQ + n, rows, :] for n in range(NTQ)], axis=1) + upd[rows, :]
            bv = jnp.concatenate([g_ref[ib * NTQ + n, rows, :] for n in range(NTQ)], axis=1)
            xs_ref[ib, rows, :] = (xs_ref[ib, rows, :].astype(f32) + sv * _silu(bv)).astype(bf16)
            cp_tail(c).start()

    def topk():
        r = jnp.concatenate([r_ref[j] for j in range(NQ)], axis=0)
        ids = (lax.broadcasted_iota(jnp.int32, (NQ, MQ), 0) * MQ
               + lax.broadcasted_iota(jnp.int32, (NQ, MQ), 1))
        rb = lax.shift_right_arithmetic(lax.bitcast_convert_type(r + 0.0, jnp.int32), 16)
        mono = jnp.where(rb < 0, -32769 - rb, rb) + 32768
        key = mono * S + (S - 1 - ids)
        keys = []
        for c in range(C):
            mx = jnp.max(jnp.max(key, axis=1, keepdims=True), axis=0, keepdims=True)
            key = jnp.where(key == mx, -1, key)
            keys.append(mx)
            idx_ref[c] = S - 1 - mx[0, 0] % S
        kv = jnp.concatenate(keys, axis=0)
        mono_s = kv // S - 32768
        rb_s = jnp.where(mono_s < 0, -32769 - mono_s, mono_s)
        rsel_ref[...] = jnp.broadcast_to(lax.bitcast_convert_type(lax.shift_left(rb_s, 16), f32), (C, 128))

    def moe():
        for cp in cp_moe():
            cp.wait()
        rows = []
        sel = []
        sub = lax.broadcasted_iota(jnp.int32, (16, DP), 0)
        for c in range(C):
            idx_s = jnp.clip(idx_ref[c], 0, S - 1)
            ib = idx_s // MQ
            off = idx_s - ib * MQ
            base = pl.multiple_of((off // 16) * 16, 16)
            blk = xn_ref[ib, pl.ds(base, 16), :].astype(f32)
            rows.append(jnp.sum(jnp.where(sub == off - base, blk, 0.0), axis=0, keepdims=True))
            sel.append(idx_s)
        rsel = rsel_ref[:, 0:1]
        xsel = jnp.concatenate(rows, axis=0)
        xs16 = jnp.concatenate([xsel, xsel], axis=0)[:, :D].astype(bf16)
        gt = _rb(jnp.dot(xs16, wg_ref[...], preferred_element_type=f32))
        u = _rb(jnp.dot(xs16, wu_ref[...], preferred_element_type=f32))
        hh = (_rb(_silu(gt)) * u).astype(bf16)
        y = _rb(lax.dot_general(hh, wdt_ref[...], NT, preferred_element_type=f32))[:C]
        y = _rb(y * _rb(_sigmoid(rsel)))
        gsel = _rb(xsel[:, :D] + y)
        gpad = jnp.concatenate([gsel, jnp.zeros((C, DP - D), f32)], axis=1)
        gpad = jnp.concatenate([gpad, jnp.zeros((128 - C, DP), f32)], axis=0)
        gt_all = gpad.T[:D]
        lane = lax.broadcasted_iota(jnp.int32, (D, 128), 1)
        for c in range(C):
            idx_s = sel[c]
            tt = idx_s // 128
            g_ref[tt] = jnp.where(lane == idx_s - tt * 128, gt_all[:, c:c + 1], g_ref[tt])

    def main_block(t, carry, first=False, last=False):
        h = t // NQ
        i = t % NQ
        i_next = (t + 1) % NQ
        h_next = (t + 1) // NQ
        i_prev = (t - 1) % NQ
        h_prev = (t - 1) // NQ
        hv = jnp.minimum(h + 1, HKV - 1)
        z = z_ref[0]
        cur = h % 2
        st = {}
        jobs = []

        def qk(name, s_ref, col):
            q = jnp.concatenate([_upk(q_ref[col, n * 64:(n + 1) * 64, :]) for n in range(NTQ)], axis=1)
            s = jnp.dot(k_ref[h, 0:S, :], q, preferred_element_type=f32)
            for n in range(NTQ):
                s_ref[n, 0:S, :] = s[:, n * 128:(n + 1) * 128]
            m = jnp.max(s.reshape(S // 8, 8, MQ), axis=0)
            st[name] = jnp.max(m, axis=0, keepdims=True)
            jobs.append(st[name])

        def pv(name, s_ref, col):
            acc = None
            m = st[name]
            if name == "a":
                m = m + _zero_after(st["b"])
            l = None
            for j in range(S // KBP):
                kd = pl.ds(pl.multiple_of(z + j * KBP, KBP), KBP)
                sv = jnp.concatenate([s_ref[n, kd, :] for n in range(NTQ)], axis=1)
                mg = m
                if len(jobs) >= LAG:
                    mg = m + _zero_after(jobs[-LAG])
                p = jnp.exp2(sv - mg)
                lj = _tree(p, jnp.add)
                l = lj if l is None else l + lj
                pb = p.astype(bf16)
                vt = jnp.concatenate([_upk(vt_ref[cur, jj]) for jj in range(j * KBP // 128, (j + 1) * KBP // 128)], axis=1)
                oj = jnp.dot(vt, pb, preferred_element_type=f32)
                jobs.append(oj[DH - 1:DH, :])
                acc = oj if acc is None else acc + oj
            l = jnp.sum(l, axis=0, keepdims=True)
            ob = (acc * (1.0 / l)).astype(bf16)
            for n in range(NTQ):
                oc_ref[n, col * DH // 2:(col + 1) * DH // 2, :] = _pk(ob[:, n * 128:(n + 1) * 128])

        qk("a", sa_ref, 0)
        qk("b", sb_ref, 1)
        if not first:
            oproj(i_prev, h_prev, jobs)
        pv("a", sa_ref, 0)
        if last:
            epilogue(NQ - 2)
        else:
            qproj(i_next, h_next)
        pv("b", sb_ref, 1)
        if last:
            final_block()
        else:
            for jj in range(VP // 128):
                off = pl.multiple_of(i * VP + jj * 128, 128)
                vt_ref[1 - cur, i * (VP // 128) + jj] = _pk(v_ref[hv, pl.ds(off, 128), :].T)
        return carry

    def single_block(t, carry):
        topk()
        return main_block(t, carry)

    def pair_block(p, carry):
        main_block(2 * p, carry)
        main_block(2 * p + 1, carry)
        return carry

    for cp in [cp_x(0), cp_v(0), cp_wq(0), cp_x(1), cp_k(0), cp_v(1), cp_wo(0)]:
        cp.start()
    z_ref[0] = 0
    r_ref[...] = jnp.zeros(r_ref.shape, f32)

    def zero_acc(j, c):
        acc_ref[j] = jnp.zeros((D, 128), f32)
        return c
    lax.fori_loop(0, NL, zero_acc, 0)
    wr = wr_ref[...].reshape(1, D)
    wr = jnp.concatenate([wr, jnp.zeros((1, DP - D), bf16)], axis=1)
    wrow_ref[...] = jnp.broadcast_to(wr.astype(f32), (16, DP)).astype(bf16)
    cp_x(0).wait()
    layernorm_tiles(0, range(2))
    cp_v(0).wait()
    cp_wq(0).wait()
    layernorm_tiles(0, range(2, NTQ))
    for j in range(NKT):
        vt_ref[0, j] = _pk(v_ref[0, j * 128:(j + 1) * 128, :].T)
    qproj(0, 0)
    for cp in [cp_wq(1)] + [cp_x(ib) for ib in range(2, NQ)]:
        cp.start()
    for h in range(1, H_EARLY):
        for cp in group(h):
            cp.start()

    cp_x(1).wait()
    layernorm_block(1)
    cp_k(0).wait()
    cp_v(1).wait()
    main_block(0, 0, first=True)
    cp_wo(0).wait()

    starts = [1, 2] + [h * NQ for h in range(1, H_EARLY)] + [MOE_T, T - 2, T - 1]
    nseg = len(starts) - 1
    seg_moe = nseg - 2

    def segment(sg, carry):
        t0 = jnp.int32(0)
        t1 = jnp.int32(0)
        for k in range(nseg):
            t0 = jnp.where(sg == k, starts[k], t0)
            t1 = jnp.where(sg == k, starts[k + 1], t1)
        paired = jnp.logical_and(sg >= 1, sg <= seg_moe)

        @pl.when(sg == 0)
        def _():
            for h in range(H_EARLY, HKV):
                for cp in group(h):
                    cp.start()

            def ln(ib, c):
                cp_x(ib).wait()
                layernorm_block(ib)
                return c
            lax.fori_loop(2, NQ, ln, 0)

        @pl.when(sg == 1)
        def _():
            cp_wq(1).wait()

        @pl.when(sg == 1)
        def _():
            for cp in cp_moe():
                cp.start()

        for h in range(1, H_EARLY):
            @pl.when(sg == 1 + h)
            def _(h=h):
                for cp in group(h):
                    cp.wait()

        @pl.when(sg == seg_moe)
        def _():
            for h in range(H_EARLY, HKV):
                for cp in group(h):
                    cp.wait()
            moe()

        @pl.when(sg == nseg - 1)
        def _():
            epilogue(0)

        lax.fori_loop(jnp.where(paired, t0 // 2, 0), jnp.where(paired, t1 // 2, 0), pair_block, 0)
        lax.fori_loop(jnp.where(paired, 0, t0), jnp.where(paired, 0, t1), single_block, 0)
        return carry

    lax.fori_loop(0, nseg, segment, 0)

    @pl.when(z_ref[0] == 0)
    def _():
        epilogue(1)
    main_block(T - 1, 0, last=True)
    for ib in range(NQ - 1):
        cp_out(ib).wait()
    for c in range(RC):
        cp_tail(c).wait()


@jax.jit
def pallas_recurrent_scan__gqa_block_cached__moe_arch_mod__prompt_kernel(
        A_x, A_k_cache, A_v_cache, A_wq, A_wo, B_x, B_w_r, B_w_gate, B_w_up, B_w_down):
    xt = A_x.reshape(S, D).T
    anyspec = pl.BlockSpec(memory_space=pl.ANY)
    out = pl.pallas_call(
        _kernel,
        in_specs=[anyspec, anyspec, anyspec, anyspec, anyspec,
                  pl.BlockSpec(memory_space=pltpu.VMEM),
                  anyspec, anyspec, anyspec],
        out_specs=anyspec,
        out_shape=jax.ShapeDtypeStruct((D, S), bf16),
        scratch_shapes=[
            pltpu.VMEM((NQ, MQ, DP), bf16),
            pltpu.VMEM((NL, D, 128), f32),
            pltpu.VMEM((HKV, S, DH), bf16),
            pltpu.VMEM((HKV, S, DH), bf16),
            pltpu.VMEM((HKV, D, 2 * DH), bf16),
            pltpu.VMEM((HKV, D, 2 * DH), bf16),
            pltpu.VMEM((NTQ, S, 128), f32),
            pltpu.VMEM((NTQ, S, 128), f32),
            pltpu.VMEM((2, MQ // 2, DH), u32),
            pltpu.VMEM((NTQ, DH, 128), u32),
            pltpu.VMEM((2, NKT, DH // 2, 128), u32),
            pltpu.VMEM((NL, D, 128), f32),
            pltpu.VMEM((NQ, D, MQ), bf16),
            pltpu.VMEM((NQ, 1, MQ), f32),
            pltpu.VMEM((16, DP), bf16),
            pltpu.VMEM((D, F), bf16),
            pltpu.VMEM((D, F), bf16),
            pltpu.VMEM((D, F), bf16),
            pltpu.VMEM((C, 128), f32),
            pltpu.SMEM((1,), jnp.int32),
            pltpu.SMEM((C,), jnp.int32),
            pltpu.SemaphoreType.DMA((NQ,)),
            pltpu.SemaphoreType.DMA((HKV,)),
            pltpu.SemaphoreType.DMA((HKV,)),
            pltpu.SemaphoreType.DMA((HKV,)),
            pltpu.SemaphoreType.DMA((HKV,)),
            pltpu.SemaphoreType.DMA((3,)),
            pltpu.SemaphoreType.DMA((NQ,)),
            pltpu.SemaphoreType.DMA((RC,)),
        ],
        compiler_params=pltpu.CompilerParams(vmem_limit_bytes=VMEM_LIMIT),
        name="fused_attn_moe",
    )(xt, A_k_cache, A_v_cache, A_wq, A_wo.T, B_w_r, B_w_gate, B_w_up, B_w_down.T)
    return out.T.reshape(1, S, D)
```

```python
import jax
import jax.numpy as jnp
from jax import lax
import jax.experimental.pallas as pl
import jax.experimental.pallas.tpu as pltpu

S = 2048
D = 576
DP = 640
HKV = 16
DH = 128
F = 4608
C = 8
MQ = 512
KBP = 128
LAG = 5
MOE_T = 12
RC = 4
VMEM_LIMIT = 110 * 1024 * 1024

NQ = S // MQ
NL = S // 128
NTQ = MQ // 128
NKT = S // 128
VP = S // NQ
T = HKV * NQ
H_EARLY = MOE_T // NQ
QSCALE = (DH ** -0.5) * 1.4426950408889634

bf16 = jnp.bfloat16
f32 = jnp.float32
u32 = jnp.uint32
NT = (((1,), (1,)), ((), ()))


def _rb(x):
    return x.astype(bf16).astype(f32)


def _pk(x):
    return pltpu.bitcast(x, u32)


def _upk(x):
    return pltpu.bitcast(x, bf16)


def _sigmoid(x):
    return 0.5 * jnp.tanh(0.5 * x) + 0.5


def _silu(x):
    h = 0.5 * x
    return h * jnp.tanh(h) + h


def _lin(p, op, n=2):
    parts = [p[i * 8:(i + 1) * 8] for i in range(p.shape[0] // 8)]
    acc = parts[:n]
    for i in range(n, len(parts)):
        acc[i % n] = op(acc[i % n], parts[i])
    while len(acc) > 1:
        acc = [op(acc[i], acc[i + 1]) for i in range(0, len(acc), 2)]
    return acc[0]


def _tree(p, op):
    parts = [p[i * 8:(i + 1) * 8] for i in range(p.shape[0] // 8)]
    while len(parts) > 1:
        nxt = [op(parts[i], parts[i + 1]) for i in range(0, len(parts) - 1, 2)]
        if len(parts) % 2:
            nxt.append(parts[-1])
        parts = nxt
    return parts[0]


def _zero_after(x):
    return jnp.minimum(jnp.abs(x), 0.0)


def _kernel(xt_hbm, k_hbm, v_hbm, wq_hbm, wot_hbm, wr_ref, wg_hbm, wu_hbm, wdt_hbm,
            o_hbm,
            xn_ref, acc_ref, k_ref, v_ref, wq_ref, wo_ref,
            sa_ref, sb_ref, q_ref, oc_ref, vt_ref,
            g_ref, xs_ref, r_ref, wrow_ref, wg_ref, wu_ref, wdt_ref, rsel_ref, z_ref, idx_ref,
            sem_x, sem_k, sem_v, sem_wq, sem_wo, sem_m, sem_o, sem_t):

    def cp_x(ib):
        return pltpu.make_async_copy(xt_hbm.at[:, pl.ds(ib * MQ, MQ)], xs_ref.at[ib], sem_x.at[ib])

    def cp_k(h):
        return pltpu.make_async_copy(k_hbm.at[0, h], k_ref.at[h], sem_k.at[h])

    def cp_v(h):
        return pltpu.make_async_copy(v_hbm.at[0, h], v_ref.at[h], sem_v.at[h])

    def cp_wq(h):
        return pltpu.make_async_copy(wq_hbm.at[:, pl.ds(h * 256, 256)], wq_ref.at[h], sem_wq.at[h])

    def cp_wo(h):
        return pltpu.make_async_copy(wot_hbm.at[:, pl.ds(h * 256, 256)], wo_ref.at[h], sem_wo.at[h])

    def cp_moe():
        return [pltpu.make_async_copy(wg_hbm, wg_ref, sem_m.at[0]),
                pltpu.make_async_copy(wu_hbm, wu_ref, sem_m.at[1]),
                pltpu.make_async_copy(wdt_hbm, wdt_ref, sem_m.at[2])]

    def cp_out(ib):
        return pltpu.make_async_copy(xs_ref.at[ib], o_hbm.at[:, pl.ds(pl.multiple_of(ib * MQ, MQ), MQ)], sem_o.at[ib])

    def cp_tail(c):
        rr = D // RC
        return pltpu.make_async_copy(xs_ref.at[NQ - 1, pl.ds(c * rr, rr)],
                                     o_hbm.at[pl.ds(c * rr, rr), pl.ds((NQ - 1) * MQ, MQ)], sem_t.at[c])

    def group(h):
        cps = [cp_k(h), cp_wo(h)]
        if h + 1 < HKV:
            cps += [cp_v(h + 1), cp_wq(h + 1)]
        return cps

    def bulk():
        nk = HKV - H_EARLY
        cps = [pltpu.make_async_copy(k_hbm.at[0, pl.ds(H_EARLY, nk)], k_ref.at[pl.ds(H_EARLY, nk)], sem_k.at[H_EARLY]),
               pltpu.make_async_copy(v_hbm.at[0, pl.ds(H_EARLY + 1, nk - 1)], v_ref.at[pl.ds(H_EARLY + 1, nk - 1)],
                                     sem_v.at[H_EARLY + 1])]
        for h in range(H_EARLY, HKV):
            cps.append(cp_wo(h))
            if h + 1 < HKV:
                cps.append(cp_wq(h + 1))
        return cps

    def layernorm_tiles(ib, tiles):
        wrow = wrow_ref[...]
        for j in tiles:
            x = xs_ref[ib, :, j * 128:(j + 1) * 128].astype(f32)
            mean = jnp.sum(_lin(x, jnp.add), axis=0, keepdims=True) * (1.0 / D)
            xc = x - mean
            var = jnp.sum(_lin(xc * xc, jnp.add), axis=0, keepdims=True) * (1.0 / D)
            m = _rb(mean)
            inv = 1.0 / _rb(jnp.sqrt(_rb(_rb(var) + 1e-5)))
            xn = _rb(x - m) * inv
            g_ref[ib * NTQ + j] = xn
            xnp = jnp.concatenate([xn, jnp.zeros((DP - D, 128), f32)], axis=0).astype(bf16)
            r_ref[ib, :, j * 128:(j + 1) * 128] = _rb(jnp.dot(wrow, xnp, preferred_element_type=f32)[0:1, :])
            xn_ref[ib, j * 128:(j + 1) * 128, :] = xnp.T

    def layernorm_block(ib):
        layernorm_tiles(ib, range(NTQ))

    def qproj(ib, hh):
        xn = xn_ref[ib][:, :D]
        q = jnp.dot(xn, wq_ref[hh], preferred_element_type=f32) * QSCALE
        q = q.astype(bf16)
        for hh2 in range(2):
            for n in range(NTQ):
                q_ref[hh2, n * 64:(n + 1) * 64, :] = _pk(q[n * 128:(n + 1) * 128, hh2 * DH:(hh2 + 1) * DH].T)

    def oproj(ib, hh, jobs):
        upd = jnp.dot(wo_ref[hh], jnp.concatenate([_upk(oc_ref[n]) for n in range(NTQ)], axis=1),
                      preferred_element_type=f32)
        jobs.append(upd[D - 1:D, :])
        for n in range(NTQ):
            acc_ref[ib * NTQ + n] = acc_ref[ib * NTQ + n] + upd[:, n * 128:(n + 1) * 128]

    def epilogue(ib):
        sv = jnp.concatenate([acc_ref[ib * NTQ + j] for j in range(NTQ)], axis=1)
        bv = jnp.concatenate([g_ref[ib * NTQ + j] for j in range(NTQ)], axis=1)
        xs_ref[ib] = (xs_ref[ib].astype(f32) + sv * _silu(bv)).astype(bf16)
        cp_out(ib).start()

    def final_block():
        ib = NQ - 1
        upd = jnp.dot(wo_ref[HKV - 1], jnp.concatenate([_upk(oc_ref[n]) for n in range(NTQ)], axis=1),
                      preferred_element_type=f32)
        rr = D // RC
        for c in range(RC):
            rows = slice(c * rr, (c + 1) * rr)
            sv = jnp.concatenate([acc_ref[ib * NTQ + n, rows, :] for n in range(NTQ)], axis=1) + upd[rows, :]
            bv = jnp.concatenate([g_ref[ib * NTQ + n, rows, :] for n in range(NTQ)], axis=1)
            xs_ref[ib, rows, :] = (xs_ref[ib, rows, :].astype(f32) + sv * _silu(bv)).astype(bf16)
            cp_tail(c).start()

    def topk():
        r = jnp.concatenate([r_ref[j] for j in range(NQ)], axis=0)
        ids = (lax.broadcasted_iota(jnp.int32, (NQ, MQ), 0) * MQ
               + lax.broadcasted_iota(jnp.int32, (NQ, MQ), 1))
        rb = lax.shift_right_arithmetic(lax.bitcast_convert_type(r + 0.0, jnp.int32), 16)
        mono = jnp.where(rb < 0, -32769 - rb, rb) + 32768
        key = mono * S + (S - 1 - ids)
        keys = []
        for c in range(C):
            mx = jnp.max(jnp.max(key, axis=1, keepdims=True), axis=0, keepdims=True)
            key = jnp.where(key == mx, -1, key)
            keys.append(mx)
            idx_ref[c] = S - 1 - mx[0, 0] % S
        kv = jnp.concatenate(keys, axis=0)
        mono_s = kv // S - 32768
        rb_s = jnp.where(mono_s < 0, -32769 - mono_s, mono_s)
        rsel_ref[...] = jnp.broadcast_to(lax.bitcast_convert_type(lax.shift_left(rb_s, 16), f32), (C, 128))

    def moe():
        for cp in cp_moe():
            cp.wait()
        rows = []
        sel = []
        sub = lax.broadcasted_iota(jnp.int32, (16, DP), 0)
        for c in range(C):
            idx_s = jnp.clip(idx_ref[c], 0, S - 1)
            ib = idx_s // MQ
            off = idx_s - ib * MQ
            base = pl.multiple_of((off // 16) * 16, 16)
            blk = xn_ref[ib, pl.ds(base, 16), :].astype(f32)
            rows.append(jnp.sum(jnp.where(sub == off - base, blk, 0.0), axis=0, keepdims=True))
            sel.append(idx_s)
        rsel = rsel_ref[:, 0:1]
        xsel = jnp.concatenate(rows, axis=0)
        xs16 = jnp.concatenate([xsel, xsel], axis=0)[:, :D].astype(bf16)
        gt = _rb(jnp.dot(xs16, wg_ref[...], preferred_element_type=f32))
        u = _rb(jnp.dot(xs16, wu_ref[...], preferred_element_type=f32))
        hh = (_rb(_silu(gt)) * u).astype(bf16)
        y = _rb(lax.dot_general(hh, wdt_ref[...], NT, preferred_element_type=f32))[:C]
        y = _rb(y * _rb(_sigmoid(rsel)))
        gsel = _rb(xsel[:, :D] + y)
        gpad = jnp.concatenate([gsel, jnp.zeros((C, DP - D), f32)], axis=1)
        gpad = jnp.concatenate([gpad, jnp.zeros((128 - C, DP), f32)], axis=0)
        gt_all = gpad.astype(bf16).T.astype(f32)[:D]
        lane = lax.broadcasted_iota(jnp.int32, (D, 128), 1)
        for c in range(C):
            idx_s = sel[c]
            tt = idx_s // 128
            g_ref[tt] = jnp.where(lane == idx_s - tt * 128, gt_all[:, c:c + 1], g_ref[tt])

    def main_block(t, carry, first=False, last=False):
        h = t // NQ
        i = t % NQ
        i_next = (t + 1) % NQ
        h_next = (t + 1) // NQ
        i_prev = (t - 1) % NQ
        h_prev = (t - 1) // NQ
        hv = jnp.minimum(h + 1, HKV - 1)
        z = z_ref[0]
        cur = h % 2
        st = {}
        jobs = []

        def qk(name, s_ref, col):
            q = jnp.concatenate([_upk(q_ref[col, n * 64:(n + 1) * 64, :]) for n in range(NTQ)], axis=1)
            s = jnp.dot(k_ref[h, 0:S, :], q, preferred_element_type=f32)
            for n in range(NTQ):
                s_ref[n, 0:S, :] = s[:, n * 128:(n + 1) * 128]
            m = jnp.max(s.reshape(S // 8, 8, MQ), axis=0)
            st[name] = jnp.max(m, axis=0, keepdims=True)
            jobs.append(st[name])

        def pv(name, s_ref, col):
            acc = None
            m = st[name]
            if name == "a":
                m = m + _zero_after(st["b"])
            l = None
            for j in range(S // KBP):
                kd = pl.ds(pl.multiple_of(z + j * KBP, KBP), KBP)
                sv = jnp.concatenate([s_ref[n, kd, :] for n in range(NTQ)], axis=1)
                mg = m
                if len(jobs) >= LAG:
                    mg = m + _zero_after(jobs[-LAG])
                p = jnp.exp2(sv - mg)
                lj = _tree(p, jnp.add)
                l = lj if l is None else l + lj
                pb = p.astype(bf16)
                vt = jnp.concatenate([_upk(vt_ref[cur, jj]) for jj in range(j * KBP // 128, (j + 1) * KBP // 128)], axis=1)
                oj = jnp.dot(vt, pb, preferred_element_type=f32)
                jobs.append(oj[DH - 1:DH, :])
                acc = oj if acc is None else acc + oj
            l = jnp.sum(l, axis=0, keepdims=True)
            ob = (acc * (1.0 / l)).astype(bf16)
            for n in range(NTQ):
                oc_ref[n, col * DH // 2:(col + 1) * DH // 2, :] = _pk(ob[:, n * 128:(n + 1) * 128])

        qk("a", sa_ref, 0)
        qk("b", sb_ref, 1)
        if not first:
            oproj(i_prev, h_prev, jobs)
        pv("a", sa_ref, 0)
        if last:
            epilogue(NQ - 2)
        else:
            qproj(i_next, h_next)
        pv("b", sb_ref, 1)
        if last:
            final_block()
        else:
            for jj in range(VP // 128):
                off = pl.multiple_of(i * VP + jj * 128, 128)
                vt_ref[1 - cur, i * (VP // 128) + jj] = _pk(v_ref[hv, pl.ds(off, 128), :].T)
        return carry

    def single_block(t, carry):
        topk()
        return main_block(t, carry)

    def pair_block(p, carry):
        main_block(2 * p, carry)
        main_block(2 * p + 1, carry)
        return carry

    for cp in [cp_x(0), cp_v(0), cp_wq(0), cp_x(1), cp_k(0), cp_v(1), cp_wo(0)]:
        cp.start()
    z_ref[0] = 0
    r_ref[...] = jnp.zeros(r_ref.shape, f32)

    def zero_acc(j, c):
        acc_ref[j] = jnp.zeros((D, 128), f32)
        return c
    lax.fori_loop(0, NL, zero_acc, 0)
    wr = wr_ref[...].reshape(1, D)
    wr = jnp.concatenate([wr, jnp.zeros((1, DP - D), bf16)], axis=1)
    wrow_ref[...] = jnp.broadcast_to(wr.astype(f32), (16, DP)).astype(bf16)
    cp_x(0).wait()
    layernorm_tiles(0, range(2))
    cp_v(0).wait()
    cp_wq(0).wait()
    layernorm_tiles(0, range(2, NTQ))
    for j in range(NKT):
        vt_ref[0, j] = _pk(v_ref[0, j * 128:(j + 1) * 128, :].T)
    qproj(0, 0)
    for cp in [cp_wq(1)] + [cp_x(ib) for ib in range(2, NQ)]:
        cp.start()
    for h in range(1, H_EARLY):
        for cp in group(h):
            cp.start()

    cp_x(1).wait()
    layernorm_block(1)
    cp_k(0).wait()
    cp_v(1).wait()
    main_block(0, 0, first=True)
    cp_wo(0).wait()

    starts = [1, 2] + [h * NQ for h in range(1, H_EARLY)] + [MOE_T, T - 2, T - 1]
    nseg = len(starts) - 1
    seg_moe = nseg - 2

    def segment(sg, carry):
        t0 = jnp.int32(0)
        t1 = jnp.int32(0)
        for k in range(nseg):
            t0 = jnp.where(sg == k, starts[k], t0)
            t1 = jnp.where(sg == k, starts[k + 1], t1)
        paired = jnp.logical_and(sg >= 1, sg <= seg_moe)

        @pl.when(sg == 0)
        def _():
            for cp in bulk():
                cp.start()

            def ln(ib, c):
                cp_x(ib).wait()
                layernorm_block(ib)
                return c
            lax.fori_loop(2, NQ, ln, 0)

        @pl.when(sg == 1)
        def _():
            cp_wq(1).wait()

        @pl.when(sg == 1)
        def _():
            for cp in cp_moe():
                cp.start()

        for h in range(1, H_EARLY):
            @pl.when(sg == 1 + h)
            def _(h=h):
                for cp in group(h):
                    cp.wait()

        @pl.when(sg == seg_moe)
        def _():
            for cp in bulk():
                cp.wait()
            moe()

        @pl.when(sg == nseg - 1)
        def _():
            epilogue(0)

        lax.fori_loop(jnp.where(paired, t0 // 2, 0), jnp.where(paired, t1 // 2, 0), pair_block, 0)
        lax.fori_loop(jnp.where(paired, 0, t0), jnp.where(paired, 0, t1), single_block, 0)
        return carry

    lax.fori_loop(0, nseg, segment, 0)

    @pl.when(z_ref[0] == 0)
    def _():
        epilogue(1)
    main_block(T - 1, 0, last=True)
    for ib in range(NQ - 1):
        cp_out(ib).wait()
    for c in range(RC):
        cp_tail(c).wait()


@jax.jit
def pallas_recurrent_scan__gqa_block_cached__moe_arch_mod__prompt_kernel(
        A_x, A_k_cache, A_v_cache, A_wq, A_wo, B_x, B_w_r, B_w_gate, B_w_up, B_w_down):
    xt = A_x.reshape(S, D).T
    anyspec = pl.BlockSpec(memory_space=pl.ANY)
    out = pl.pallas_call(
        _kernel,
        in_specs=[anyspec, anyspec, anyspec, anyspec, anyspec,
                  pl.BlockSpec(memory_space=pltpu.VMEM),
                  anyspec, anyspec, anyspec],
        out_specs=anyspec,
        out_shape=jax.ShapeDtypeStruct((D, S), bf16),
        scratch_shapes=[
            pltpu.VMEM((NQ, MQ, DP), bf16),
            pltpu.VMEM((NL, D, 128), f32),
            pltpu.VMEM((HKV, S, DH), bf16),
            pltpu.VMEM((HKV, S, DH), bf16),
            pltpu.VMEM((HKV, D, 2 * DH), bf16),
            pltpu.VMEM((HKV, D, 2 * DH), bf16),
            pltpu.VMEM((NTQ, S, 128), f32),
            pltpu.VMEM((NTQ, S, 128), f32),
            pltpu.VMEM((2, MQ // 2, DH), u32),
            pltpu.VMEM((NTQ, DH, 128), u32),
            pltpu.VMEM((2, NKT, DH // 2, 128), u32),
            pltpu.VMEM((NL, D, 128), f32),
            pltpu.VMEM((NQ, D, MQ), bf16),
            pltpu.VMEM((NQ, 1, MQ), f32),
            pltpu.VMEM((16, DP), bf16),
            pltpu.VMEM((D, F), bf16),
            pltpu.VMEM((D, F), bf16),
            pltpu.VMEM((D, F), bf16),
            pltpu.VMEM((C, 128), f32),
            pltpu.SMEM((1,), jnp.int32),
            pltpu.SMEM((C,), jnp.int32),
            pltpu.SemaphoreType.DMA((NQ,)),
            pltpu.SemaphoreType.DMA((HKV,)),
            pltpu.SemaphoreType.DMA((HKV,)),
            pltpu.SemaphoreType.DMA((HKV,)),
            pltpu.SemaphoreType.DMA((HKV,)),
            pltpu.SemaphoreType.DMA((3,)),
            pltpu.SemaphoreType.DMA((NQ,)),
            pltpu.SemaphoreType.DMA((RC,)),
        ],
        compiler_params=pltpu.CompilerParams(vmem_limit_bytes=VMEM_LIMIT),
        name="fused_attn_moe",
    )(xt, A_k_cache, A_v_cache, A_wq, A_wo.T, B_w_r, B_w_gate, B_w_up, B_w_down.T)
    return out.T.reshape(1, S, D)
```

```python
import jax
import jax.numpy as jnp
from jax import lax
import jax.experimental.pallas as pl
import jax.experimental.pallas.tpu as pltpu

S = 2048
D = 576
DP = 640
HKV = 16
DH = 128
F = 4608
C = 8
MQ = 512
KBP = 128
LAG = 5
MOE_T = 12
RC = 4
VMEM_LIMIT = 110 * 1024 * 1024

NQ = S // MQ
NL = S // 128
NTQ = MQ // 128
NKT = S // 128
VP = S // NQ
T = HKV * NQ
H_EARLY = MOE_T // NQ
QSCALE = (DH ** -0.5) * 1.4426950408889634

bf16 = jnp.bfloat16
f32 = jnp.float32
u32 = jnp.uint32
NT = (((1,), (1,)), ((), ()))


def _rb(x):
    return x.astype(bf16).astype(f32)


def _pk(x):
    return pltpu.bitcast(x, u32)


def _upk(x):
    return pltpu.bitcast(x, bf16)


def _sigmoid(x):
    return 0.5 * jnp.tanh(0.5 * x) + 0.5


def _silu(x):
    h = 0.5 * x
    return h * jnp.tanh(h) + h


def _lin(p, op, n=2):
    parts = [p[i * 8:(i + 1) * 8] for i in range(p.shape[0] // 8)]
    acc = parts[:n]
    for i in range(n, len(parts)):
        acc[i % n] = op(acc[i % n], parts[i])
    while len(acc) > 1:
        acc = [op(acc[i], acc[i + 1]) for i in range(0, len(acc), 2)]
    return acc[0]


def _tree(p, op):
    parts = [p[i * 8:(i + 1) * 8] for i in range(p.shape[0] // 8)]
    while len(parts) > 1:
        nxt = [op(parts[i], parts[i + 1]) for i in range(0, len(parts) - 1, 2)]
        if len(parts) % 2:
            nxt.append(parts[-1])
        parts = nxt
    return parts[0]


def _zero_after(x):
    return jnp.minimum(jnp.abs(x), 0.0)


def _kernel(xt_hbm, k_hbm, v_hbm, wq_hbm, wot_hbm, wr_ref, wg_hbm, wu_hbm, wdt_hbm,
            o_hbm,
            xn_ref, acc_ref, k_ref, v_ref, wq_ref, wo_ref,
            sa_ref, sb_ref, q_ref, oc_ref, vt_ref,
            g_ref, xs_ref, r_ref, wrow_ref, wg_ref, wu_ref, wdt_ref, rsel_ref, z_ref, idx_ref,
            sem_x, sem_k, sem_v, sem_wq, sem_wo, sem_m, sem_o, sem_t):

    def cp_x(ib):
        return pltpu.make_async_copy(xt_hbm.at[:, pl.ds(ib * MQ, MQ)], xs_ref.at[ib], sem_x.at[ib])

    def cp_k(h):
        return pltpu.make_async_copy(k_hbm.at[0, h], k_ref.at[h], sem_k.at[h])

    def cp_v(h):
        return pltpu.make_async_copy(v_hbm.at[0, h], v_ref.at[h], sem_v.at[h])

    def cp_wq(h):
        return pltpu.make_async_copy(wq_hbm.at[:, pl.ds(h * 256, 256)], wq_ref.at[h], sem_wq.at[h])

    def cp_wo(h):
        return pltpu.make_async_copy(wot_hbm.at[:, pl.ds(h * 256, 256)], wo_ref.at[h], sem_wo.at[h])

    def cp_moe():
        return [pltpu.make_async_copy(wg_hbm, wg_ref, sem_m.at[0]),
                pltpu.make_async_copy(wu_hbm, wu_ref, sem_m.at[1]),
                pltpu.make_async_copy(wdt_hbm, wdt_ref, sem_m.at[2])]

    def cp_out(ib):
        return pltpu.make_async_copy(xs_ref.at[ib], o_hbm.at[:, pl.ds(pl.multiple_of(ib * MQ, MQ), MQ)], sem_o.at[ib])

    def cp_tail(c):
        rr = D // RC
        return pltpu.make_async_copy(xs_ref.at[NQ - 1, pl.ds(c * rr, rr)],
                                     o_hbm.at[pl.ds(c * rr, rr), pl.ds((NQ - 1) * MQ, MQ)], sem_t.at[c])

    def group(h):
        cps = [cp_k(h), cp_wo(h)]
        if h + 1 < HKV:
            cps += [cp_v(h + 1), cp_wq(h + 1)]
        return cps

    def bulk():
        nk = HKV - H_EARLY
        cps = [pltpu.make_async_copy(k_hbm.at[0, pl.ds(H_EARLY, nk)], k_ref.at[pl.ds(H_EARLY, nk)], sem_k.at[H_EARLY]),
               pltpu.make_async_copy(v_hbm.at[0, pl.ds(H_EARLY + 1, nk - 1)], v_ref.at[pl.ds(H_EARLY + 1, nk - 1)],
                                     sem_v.at[H_EARLY + 1])]
        for h in range(H_EARLY, HKV):
            cps.append(cp_wo(h))
            if h + 1 < HKV:
                cps.append(cp_wq(h + 1))
        return cps

    def layernorm_tiles(ib, tiles, defer=None):
        wrow = wrow_ref[...]
        for j in tiles:
            x = xs_ref[ib, :, j * 128:(j + 1) * 128].astype(f32)
            mean = jnp.sum(_lin(x, jnp.add), axis=0, keepdims=True) * (1.0 / D)
            xc = x - mean
            var = jnp.sum(_lin(xc * xc, jnp.add), axis=0, keepdims=True) * (1.0 / D)
            m = _rb(mean)
            inv = 1.0 / _rb(jnp.sqrt(_rb(_rb(var) + 1e-5)))
            xn = _rb(x - m) * inv
            g_ref[ib * NTQ + j] = xn
            xnp = jnp.concatenate([xn, jnp.zeros((DP - D, 128), f32)], axis=0).astype(bf16)

            def router(xnp=xnp, j=j):
                r_ref[ib, :, j * 128:(j + 1) * 128] = _rb(jnp.dot(wrow, xnp, preferred_element_type=f32)[0:1, :])
            if defer is None:
                router()
            else:
                defer.append(router)
            xn_ref[ib, j * 128:(j + 1) * 128, :] = xnp.T

    def layernorm_block(ib):
        layernorm_tiles(ib, range(NTQ))

    def qproj(ib, hh):
        xn = xn_ref[ib][:, :D]
        q = jnp.dot(xn, wq_ref[hh], preferred_element_type=f32) * QSCALE
        q = q.astype(bf16)
        for hh2 in range(2):
            for n in range(NTQ):
                q_ref[hh2, n * 64:(n + 1) * 64, :] = _pk(q[n * 128:(n + 1) * 128, hh2 * DH:(hh2 + 1) * DH].T)

    def oproj(ib, hh, jobs):
        upd = jnp.dot(wo_ref[hh], jnp.concatenate([_upk(oc_ref[n]) for n in range(NTQ)], axis=1),
                      preferred_element_type=f32)
        jobs.append(upd[D - 1:D, :])
        for n in range(NTQ):
            acc_ref[ib * NTQ + n] = acc_ref[ib * NTQ + n] + upd[:, n * 128:(n + 1) * 128]

    def epilogue(ib):
        sv = jnp.concatenate([acc_ref[ib * NTQ + j] for j in range(NTQ)], axis=1)
        bv = jnp.concatenate([g_ref[ib * NTQ + j] for j in range(NTQ)], axis=1)
        xs_ref[ib] = (xs_ref[ib].astype(f32) + sv * _silu(bv)).astype(bf16)
        cp_out(ib).start()

    def final_block():
        ib = NQ - 1
        upd = jnp.dot(wo_ref[HKV - 1], jnp.concatenate([_upk(oc_ref[n]) for n in range(NTQ)], axis=1),
                      preferred_element_type=f32)
        rr = D // RC
        for c in range(RC):
            rows = slice(c * rr, (c + 1) * rr)
            sv = jnp.concatenate([acc_ref[ib * NTQ + n, rows, :] for n in range(NTQ)], axis=1) + upd[rows, :]
            bv = jnp.concatenate([g_ref[ib * NTQ + n, rows, :] for n in range(NTQ)], axis=1)
            xs_ref[ib, rows, :] = (xs_ref[ib, rows, :].astype(f32) + sv * _silu(bv)).astype(bf16)
            cp_tail(c).start()

    def topk():
        r = jnp.concatenate([r_ref[j] for j in range(NQ)], axis=0)
        ids = (lax.broadcasted_iota(jnp.int32, (NQ, MQ), 0) * MQ
               + lax.broadcasted_iota(jnp.int32, (NQ, MQ), 1))
        rb = lax.shift_right_arithmetic(lax.bitcast_convert_type(r + 0.0, jnp.int32), 16)
        mono = jnp.where(rb < 0, -32769 - rb, rb) + 32768
        key = mono * S + (S - 1 - ids)
        keys = []
        for c in range(C):
            mx = jnp.max(jnp.max(key, axis=1, keepdims=True), axis=0, keepdims=True)
            key = jnp.where(key == mx, -1, key)
            keys.append(mx)
            idx_ref[c] = S - 1 - mx[0, 0] % S
        kv = jnp.concatenate(keys, axis=0)
        mono_s = kv // S - 32768
        rb_s = jnp.where(mono_s < 0, -32769 - mono_s, mono_s)
        rsel_ref[...] = jnp.broadcast_to(lax.bitcast_convert_type(lax.shift_left(rb_s, 16), f32), (C, 128))

    def moe():
        for cp in cp_moe():
            cp.wait()
        rows = []
        sel = []
        sub = lax.broadcasted_iota(jnp.int32, (16, DP), 0)
        for c in range(C):
            idx_s = jnp.clip(idx_ref[c], 0, S - 1)
            ib = idx_s // MQ
            off = idx_s - ib * MQ
            base = pl.multiple_of((off // 16) * 16, 16)
            blk = xn_ref[ib, pl.ds(base, 16), :].astype(f32)
            rows.append(jnp.sum(jnp.where(sub == off - base, blk, 0.0), axis=0, keepdims=True))
            sel.append(idx_s)
        rsel = rsel_ref[:, 0:1]
        xsel = jnp.concatenate(rows, axis=0)
        xs16 = jnp.concatenate([xsel, xsel], axis=0)[:, :D].astype(bf16)
        gt = _rb(jnp.dot(xs16, wg_ref[...], preferred_element_type=f32))
        u = _rb(jnp.dot(xs16, wu_ref[...], preferred_element_type=f32))
        hh = (_rb(_silu(gt)) * u).astype(bf16)
        y = _rb(lax.dot_general(hh, wdt_ref[...], NT, preferred_element_type=f32))[:C]
        y = _rb(y * _rb(_sigmoid(rsel)))
        gsel = _rb(xsel[:, :D] + y)
        gpad = jnp.concatenate([gsel, jnp.zeros((C, DP - D), f32)], axis=1)
        gpad = jnp.concatenate([gpad, jnp.zeros((128 - C, DP), f32)], axis=0)
        gt_all = gpad.astype(bf16).T.astype(f32)[:D]
        lane = lax.broadcasted_iota(jnp.int32, (D, 128), 1)
        for c in range(C):
            idx_s = sel[c]
            tt = idx_s // 128
            g_ref[tt] = jnp.where(lane == idx_s - tt * 128, gt_all[:, c:c + 1], g_ref[tt])

    def main_block(t, carry, first=False, last=False):
        h = t // NQ
        i = t % NQ
        i_next = (t + 1) % NQ
        h_next = (t + 1) // NQ
        i_prev = (t - 1) % NQ
        h_prev = (t - 1) // NQ
        hv = jnp.minimum(h + 1, HKV - 1)
        z = z_ref[0]
        cur = h % 2
        st = {}
        jobs = []

        def qk(name, s_ref, col):
            q = jnp.concatenate([_upk(q_ref[col, n * 64:(n + 1) * 64, :]) for n in range(NTQ)], axis=1)
            s = jnp.dot(k_ref[h, 0:S, :], q, preferred_element_type=f32)
            for n in range(NTQ):
                s_ref[n, 0:S, :] = s[:, n * 128:(n + 1) * 128]
            m = jnp.max(s.reshape(S // 8, 8, MQ), axis=0)
            st[name] = jnp.max(m, axis=0, keepdims=True)
            jobs.append(st[name])

        def pv(name, s_ref, col):
            acc = None
            m = st[name]
            if name == "a":
                m = m + _zero_after(st["b"])
            if name == "b" and "ln" in st:
                m = m + st["ln"]
            l = None
            for j in range(S // KBP):
                kd = pl.ds(pl.multiple_of(z + j * KBP, KBP), KBP)
                sv = jnp.concatenate([s_ref[n, kd, :] for n in range(NTQ)], axis=1)
                mg = m
                if len(jobs) >= LAG:
                    mg = m + _zero_after(jobs[-LAG])
                p = jnp.exp2(sv - mg)
                lj = _tree(p, jnp.add)
                l = lj if l is None else l + lj
                pb = p.astype(bf16)
                vt = jnp.concatenate([_upk(vt_ref[cur, jj]) for jj in range(j * KBP // 128, (j + 1) * KBP // 128)], axis=1)
                oj = jnp.dot(vt, pb, preferred_element_type=f32)
                jobs.append(oj[DH - 1:DH, :])
                acc = oj if acc is None else acc + oj
            l = jnp.sum(l, axis=0, keepdims=True)
            ob = (acc * (1.0 / l)).astype(bf16)
            for n in range(NTQ):
                oc_ref[n, col * DH // 2:(col + 1) * DH // 2, :] = _pk(ob[:, n * 128:(n + 1) * 128])

        qk("a", sa_ref, 0)
        if first:
            cp_v(0).wait()
            cp_x(1).wait()
            for ib in range(2, NQ):
                cp_x(ib).start()
            for j in range(NKT):
                vt_ref[0, j] = _pk(v_ref[0, j * 128:(j + 1) * 128, :].T)
            routers = []
            layernorm_tiles(1, range(NTQ), routers)
            t1 = jnp.concatenate([g_ref[NTQ + j + z, 0:1, :] for j in range(NTQ)], axis=1)
            t2 = xn_ref[1 + z, 0:16, 0:128].astype(f32)[0:1, :]
            st["ln"] = _zero_after(t1) + jnp.concatenate([_zero_after(t2)] * NTQ, axis=1)
        qk("b", sb_ref, 1)
        if not first:
            oproj(i_prev, h_prev, jobs)
        pv("a", sa_ref, 0)
        if first:
            for f in routers:
                f()
        if last:
            epilogue(NQ - 2)
        else:
            qproj(i_next, h_next)
        if first:
            cp_v(1).wait()
            cp_wq(1).start()
            for hh in range(1, H_EARLY):
                for cp in group(hh):
                    cp.start()
        pv("b", sb_ref, 1)
        if last:
            final_block()
        else:
            for jj in range(VP // 128):
                off = pl.multiple_of(i * VP + jj * 128, 128)
                vt_ref[1 - cur, i * (VP // 128) + jj] = _pk(v_ref[hv, pl.ds(off, 128), :].T)
        return carry

    def single_block(t, carry):
        topk()
        return main_block(t, carry)

    def pair_block(p, carry):
        main_block(2 * p, carry)
        main_block(2 * p + 1, carry)
        return carry

    for cp in [cp_x(0), cp_wq(0)]:
        cp.start()
    z_ref[0] = 0
    r_ref[...] = jnp.zeros(r_ref.shape, f32)

    def zero_acc(j, c):
        acc_ref[j] = jnp.zeros((D, 128), f32)
        return c
    lax.fori_loop(0, NL, zero_acc, 0)
    wr = wr_ref[...].reshape(1, D)
    wr = jnp.concatenate([wr, jnp.zeros((1, DP - D), bf16)], axis=1)
    wrow_ref[...] = jnp.broadcast_to(wr.astype(f32), (16, DP)).astype(bf16)
    cp_x(0).wait()
    cp_k(0).start()
    layernorm_tiles(0, range(2))
    cp_wq(0).wait()
    cp_v(0).start()
    cp_x(1).start()
    layernorm_tiles(0, range(2, NTQ))
    qproj(0, 0)

    cp_k(0).wait()
    cp_v(1).start()
    cp_wo(0).start()
    main_block(0, 0, first=True)
    cp_wo(0).wait()

    starts = [1, 2] + [h * NQ for h in range(1, H_EARLY)] + [MOE_T, T - 2, T - 1]
    nseg = len(starts) - 1
    seg_moe = nseg - 2

    def segment(sg, carry):
        t0 = jnp.int32(0)
        t1 = jnp.int32(0)
        for k in range(nseg):
            t0 = jnp.where(sg == k, starts[k], t0)
            t1 = jnp.where(sg == k, starts[k + 1], t1)
        paired = jnp.logical_and(sg >= 1, sg <= seg_moe)

        @pl.when(sg == 0)
        def _():
            for cp in bulk():
                cp.start()

            def ln(ib, c):
                cp_x(ib).wait()
                layernorm_block(ib)
                return c
            lax.fori_loop(2, NQ, ln, 0)

        @pl.when(sg == 1)
        def _():
            cp_wq(1).wait()

        @pl.when(sg == 1)
        def _():
            for cp in cp_moe():
                cp.start()

        for h in range(1, H_EARLY):
            @pl.when(sg == 1 + h)
            def _(h=h):
                for cp in group(h):
                    cp.wait()

        @pl.when(sg == seg_moe)
        def _():
            for cp in bulk():
                cp.wait()
            moe()

        @pl.when(sg == nseg - 1)
        def _():
            epilogue(0)

        lax.fori_loop(jnp.where(paired, t0 // 2, 0), jnp.where(paired, t1 // 2, 0), pair_block, 0)
        lax.fori_loop(jnp.where(paired, 0, t0), jnp.where(paired, 0, t1), single_block, 0)
        return carry

    lax.fori_loop(0, nseg, segment, 0)

    @pl.when(z_ref[0] == 0)
    def _():
        epilogue(1)
    main_block(T - 1, 0, last=True)
    for ib in range(NQ - 1):
        cp_out(ib).wait()
    for c in range(RC):
        cp_tail(c).wait()


@jax.jit
def pallas_recurrent_scan__gqa_block_cached__moe_arch_mod__prompt_kernel(
        A_x, A_k_cache, A_v_cache, A_wq, A_wo, B_x, B_w_r, B_w_gate, B_w_up, B_w_down):
    xt = A_x.reshape(S, D).T
    anyspec = pl.BlockSpec(memory_space=pl.ANY)
    out = pl.pallas_call(
        _kernel,
        in_specs=[anyspec, anyspec, anyspec, anyspec, anyspec,
                  pl.BlockSpec(memory_space=pltpu.VMEM),
                  anyspec, anyspec, anyspec],
        out_specs=anyspec,
        out_shape=jax.ShapeDtypeStruct((D, S), bf16),
        scratch_shapes=[
            pltpu.VMEM((NQ, MQ, DP), bf16),
            pltpu.VMEM((NL, D, 128), f32),
            pltpu.VMEM((HKV, S, DH), bf16),
            pltpu.VMEM((HKV, S, DH), bf16),
            pltpu.VMEM((HKV, D, 2 * DH), bf16),
            pltpu.VMEM((HKV, D, 2 * DH), bf16),
            pltpu.VMEM((NTQ, S, 128), f32),
            pltpu.VMEM((NTQ, S, 128), f32),
            pltpu.VMEM((2, MQ // 2, DH), u32),
            pltpu.VMEM((NTQ, DH, 128), u32),
            pltpu.VMEM((2, NKT, DH // 2, 128), u32),
            pltpu.VMEM((NL, D, 128), f32),
            pltpu.VMEM((NQ, D, MQ), bf16),
            pltpu.VMEM((NQ, 1, MQ), f32),
            pltpu.VMEM((16, DP), bf16),
            pltpu.VMEM((D, F), bf16),
            pltpu.VMEM((D, F), bf16),
            pltpu.VMEM((D, F), bf16),
            pltpu.VMEM((C, 128), f32),
            pltpu.SMEM((1,), jnp.int32),
            pltpu.SMEM((C,), jnp.int32),
            pltpu.SemaphoreType.DMA((NQ,)),
            pltpu.SemaphoreType.DMA((HKV,)),
            pltpu.SemaphoreType.DMA((HKV,)),
            pltpu.SemaphoreType.DMA((HKV,)),
            pltpu.SemaphoreType.DMA((HKV,)),
            pltpu.SemaphoreType.DMA((3,)),
            pltpu.SemaphoreType.DMA((NQ,)),
            pltpu.SemaphoreType.DMA((RC,)),
        ],
        compiler_params=pltpu.CompilerParams(vmem_limit_bytes=VMEM_LIMIT),
        name="fused_attn_moe",
    )(xt, A_k_cache, A_v_cache, A_wq, A_wo.T, B_w_r, B_w_gate, B_w_up, B_w_down.T)
    return out.T.reshape(1, S, D)
```
